```python
import os as _os
_os.environ.setdefault("JAX_PLATFORMS", "cpu")
import jax
import jax.numpy as jnp

def _softmax(x, axis=-1):
    return jax.nn.softmax(x, axis=axis)
def _gelu(x):
    return jax.nn.gelu(x, approximate=True)
def _silu(x):
    return jax.nn.silu(x)
def _sigmoid(x):
    return jax.nn.sigmoid(x)
def _layernorm(x, axis=-1, eps=1e-5):
    m = jnp.mean(x, axis=axis, keepdims=True)
    v = jnp.var(x, axis=axis, keepdims=True)
    return (x - m) / jnp.sqrt(v + eps)
def _scatter_add(tgt, idx, src, axis=0):
    return tgt.at[idx].add(src)
def _segment_sum(src, seg, n):
    return jax.ops.segment_sum(src, seg, n)
class _Rng:
    def __init__(self, key):
        self._k = key
    def _next(self):
        self._k, sub = jax.random.split(self._k)
        return sub
    def normal(self, shape):
        return jax.random.normal(self._next(), shape, dtype=jnp.bfloat16)
    def randint(self, lo, hi, shape):
        return jax.random.randint(self._next(), shape, lo, hi, dtype=jnp.int32)
    def uniform(self, shape, lo=0.0, hi=1.0):
        return jax.random.uniform(self._next(), shape, jnp.bfloat16, lo, hi)
    def permutation(self, n):
        return jax.random.permutation(self._next(), n)


kernel_name = 'interleave_layers__ssm_conv_h3__geglu_ffn__prompt'

def setup_inputs():
    _rng = _Rng(jax.random.key(int.from_bytes(__import__("os").urandom(4), "little")))
    _w = (lambda a: (lambda t: t.astype(jnp.bfloat16) if jnp.issubdtype(t.dtype, jnp.floating) else t)(jnp.asarray(a)))
    def _A_setup():
        B, S, D = 1, 2048, 448
        ks = 4
        return {
            "q": _w((lambda *s: _rng.normal(s) * 0.05)(B, S, D)),
            "k": _w((lambda *s: _rng.normal(s) * 0.8)(B, S, D)),
            "v": _w((lambda *s: _rng.normal(s) * 0.8)(B, S, D)),
            "shift_k": _w((lambda *s: _rng.normal(s) * 0.8)(D, ks) * 0.5),
            "ssm_k": _w((lambda *s: _rng.normal(s) * 0.8)(D, S) * (1.0 / S ** 0.5)),
            "ssm_D": _w((lambda *s: _rng.normal(s) * 0.8)(D)),
        }
    _A_in = _A_setup()

    def _B_setup():
        B, S, D, F = 1, 2048, 448, 1792
        return {
            "x": _w((lambda *s: _rng.normal(s) * 0.05)(B, S, D)),
            "w_gate": _w((lambda *s: _rng.normal(s) * 0.1)(D, F)),
            "w_up": _w((lambda *s: _rng.normal(s) * 0.1)(D, F)),
            "w_down": _w((lambda *s: _rng.normal(s) * 0.1)(F, D)),
        }
    _B_in = _B_setup()

    return {
        "A_q": _A_in["q"],
        "A_k": _A_in["k"],
        "A_v": _A_in["v"],
        "A_shift_k": _A_in["shift_k"],
        "A_ssm_k": _A_in["ssm_k"],
        "A_ssm_D": _A_in["ssm_D"],
        "B_x": _B_in["x"],
        "B_w_gate": _B_in["w_gate"],
        "B_w_up": _B_in["w_up"],
        "B_w_down": _B_in["w_down"],
    }

def reference(A_q, A_k, A_v, A_shift_k, A_ssm_k, A_ssm_D, B_x, B_w_gate, B_w_up, B_w_down):
    def _A_ref(q, k, v, shift_k, ssm_k, ssm_D):
        B, S, D = q.shape
        ks = shift_k.shape[-1]
        k_pad = jnp.pad(k, ((0, 0), (ks - 1, 0), (0, 0)))
        k_shift = jnp.zeros_like(k)
        for t in range(ks):
            k_shift = k_shift + k_pad[:, t:t + S, :] * shift_k[:, ks - 1 - t][None, None, :]
        kv = k_shift * v
        L = 2 * S
        kv_pad = jnp.pad(kv, ((0, 0), (0, S), (0, 0)))
        kf_pad = jnp.pad(ssm_k, ((0, 0), (0, S)))
        kv_f = (lambda x, axes=(-2,-1): jnp.fft.rfft2(x.astype(jnp.float32), axes=axes))(kv_pad[:, None, :, :], axes=(1, 2))
        kf_f = (lambda x, axes=(-2,-1): jnp.fft.rfft2(x.astype(jnp.float32), axes=axes))(kf_pad[:, None, :], axes=(1, 2))
        kf_f = (lambda x, *d: x.transpose(*d))(kf_f, 1, 2, 0)
        y_f = kv_f * kf_f[None, :, :, :]
        y = (lambda x, s, axes=(-2,-1): jnp.fft.irfft2(x, s=s, axes=axes).astype(jnp.bfloat16))(y_f, (1, L), axes=(1, 2))[:, 0, :S, :]
        y = y + kv * ssm_D[None, None, :]
        return q * y

    def _B_ref(x, w_gate, w_up, w_down):
        return (_gelu(x @ w_gate) * (x @ w_up)) @ w_down

    x = A_q
    x = x + _A_ref(_layernorm(x, axis=-1), A_k, A_v, A_shift_k, A_ssm_k, A_ssm_D)
    x = x + _B_ref(_layernorm(x, axis=-1), B_w_gate, B_w_up, B_w_down)
    x = x + _A_ref(_layernorm(x, axis=-1), A_k, A_v, A_shift_k, A_ssm_k, A_ssm_D)
    x = x + _B_ref(_layernorm(x, axis=-1), B_w_gate, B_w_up, B_w_down)
    return x
```

```python
import contextlib
import functools
import numpy as np
import jax
import jax.numpy as jnp
import jax.experimental.pallas as pl
import jax.experimental.pallas.tpu as pltpu

F32, BF16, U32 = jnp.float32, jnp.bfloat16, jnp.uint32
LANES, HALF, SUB = 128, 64, 8
TM = 4 * LANES
FC = 2 * LANES
EPS = 1e-5
GELU_C0 = float(np.sqrt(2.0 / np.pi))
GELU_C1 = float(np.sqrt(2.0 / np.pi) * 0.044715)

LHS_TERMS = ((0, 1, 3), (2, 1, 3), (0, 0, 0), (3, 0, 0), (0, 1, 1), (2, -1, 0), (1, -1, 3))
RHS_TERMS = ((0, 1, 3), (0, 0, 0), (1, -1, 3), (2, -1, 0), (3, 0, 0), (0, 1, 1), (2, 1, 3))
OUT_TERMS = ({0: 1, 3: 1, 4: -1, 6: 1}, {2: 1, 4: 1}, {1: 1, 3: 1}, {0: 1, 1: -1, 2: 1, 5: 1})
SHORT = (3, 4, 6)
OUTER_ORDER = (2, 4, 1, 3, 0, 5, 6)
DOWN_ORDER = (2, 4, 0, 1, 5, 3, 6)


def _dft_tables():
    n = np.arange(LANES)[:, None]
    k = np.arange(LANES)[None, :]
    ang = np.pi * (((4 * k + 1) * n) % (4 * LANES)) / (2 * LANES)
    c, s = np.cos(ang), np.sin(ang)
    fwd = np.concatenate([c, s], axis=1)
    inv = np.concatenate([c.T, s.T], axis=0) / LANES
    return fwd.astype(BF16), inv.astype(BF16)


def _combo(term, quad):
    a, sign, b = term
    a = quad(a)
    b = quad(b) if sign else None
    if b is None:
        return a
    if a is None:
        assert sign > 0
        return b
    return a + b if sign > 0 else a - b


def _inner_sum(prod):
    m1, m2, m3, m4, m5, m6, m7 = (prod(s) for s in range(7))
    return [(m1 + m4) - m5 + m7, m3 + m5, m2 + m4, (m1 - m2) + m3 + m6]


def _outer_sum(prod, order, emit):
    m = {}
    for r in order:
        m[r] = prod(r)
        for quadrant, terms in enumerate(OUT_TERMS):
            if r in terms and all(x in m for x in terms):
                names = sorted(terms, key=lambda x: (x != r, terms[x] < 0))
                if terms[names[0]] < 0:
                    names[0], names[1] = names[1], names[0]
                blocks = list(m[names[0]])
                for x in names[1:]:
                    blocks = [u + v if terms[x] > 0 else u - v for u, v in zip(blocks, m[x])]
                emit(quadrant, blocks)


def _fold(x):
    x = x.reshape(x.shape[0] // (2 * SUB), 2, SUB, LANES)
    return jnp.concatenate([x[:, 0], x[:, 1]], axis=-1).astype(BF16)


def _unfold(v):
    return jnp.stack([v[:, :, :LANES], v[:, :, LANES:]], axis=1).reshape(2 * SUB * v.shape[0], LANES)


def _zip_halves(a, b):
    a, b = pltpu.bitcast(a, U32), pltpu.bitcast(b, U32)
    low = jax.lax.broadcasted_iota(jnp.int32, a.shape, 1) < HALF
    swap = pltpu.roll(jnp.where(low, b, a), HALF, 1)
    return [pltpu.bitcast(v, BF16).astype(F32) for v in (jnp.where(low, a, swap), jnp.where(low, swap, b))]


def _col_mean(x):
    return jnp.sum(x, axis=0, keepdims=True) * (1.0 / x.shape[0])


def _geglu2(gu):
    g, u = gu[:HALF], gu[HALF:]
    return (g * u) * (1.0 + jnp.tanh(g * (GELU_C0 + GELU_C1 * (g * g))))


def _kernel(q_hbm, k_hbm, v_hbm, sk_ref, h_hbm, d_ref, wg_hbm, wu_hbm, wd_hbm, fwd_ref, inv_ref,
            o_hbm,
            q_v, k_v, v_v, h_v, wg_v, wu_v, wd_v, o_v,
            coef, spec, hprev, kv_s, yf_s, y_s, wt, wgu, wd2, wd1, x_s, hc, ac2, ac1,
            marks, sems, *, opt):
    D, S = q_v.shape
    F = wg_v.shape[1]
    DH, DQ = D // 2, D // 4
    NBLK, NCH = S // TM, F // FC
    taps = sk_ref.shape[0]
    part = functools.partial

    clock = {"slot": 0, "token": None, "last": None, "no_bits": None}
    pending = {}

    def after(x):
        return link(x, clock["token"]) if opt.get("after", 1) else x

    def link(x, earlier):
        if earlier is None:
            return x
        if clock["no_bits"] is None:
            clock["no_bits"] = pltpu.bitcast(fwd_ref[0:2 * SUB, LANES:], U32)[0:1] & 0xFFFF
        bits = pltpu.bitcast(earlier, U32)[:x.shape[0]] & clock["no_bits"]
        return pltpu.bitcast(pltpu.bitcast(x, U32) | bits, x.dtype)

    def dot(a, b):
        pieces = pending.pop(clock["slot"], ())
        for n, piece in enumerate(pieces):
            if clock["last"] is not None:
                vregs = clock["last"].shape[0] // SUB
                if vregs <= 2 * SUB and opt.get("stagger", 1):
                    row = (clock["slot"] % 4 * len(pieces) + n) * vregs // (4 * len(pieces)) * SUB
                else:
                    row = n * vregs // len(pieces) * SUB
                clock["token"] = clock["last"][row:row + SUB, :LANES]
            piece()
        clock["slot"] += 1
        clock["last"] = jnp.dot(a(), b(), preferred_element_type=F32)
        return clock["last"]

    def tile(j):
        return slice(j * LANES, (j + 1) * LANES)

    sem_ids, in_flight = {}, []

    def copies(name):
        kind, n = name[0], name[1]
        if kind == "head":
            views = [(p, (slice(n * DH, (n + 1) * DH), slice(0, TM))) for p in ((h_hbm, h_v), (k_hbm, k_v), (v_hbm, v_v))]
        elif kind == "conv":
            cols = slice(TM, 2 * TM) if n == 1 else slice(2 * TM, S)
            views = [(p, (slice(None), cols)) for p in ((k_hbm, k_v), (v_hbm, v_v), (h_hbm, h_v))]
        elif kind == "q":
            views = [((q_hbm, q_v), (slice(None), slice(0, TM) if n == 0 else slice(TM, S)))]
        elif kind == "w":
            views = [(p, (slice(None), slice(n * FC, (n + 1) * FC))) for p in ((wg_hbm, wg_v), (wu_hbm, wu_v))]
        elif kind == "wd":
            views = [((wd_hbm, wd_v), (slice(None), slice(None)))]
        else:
            i, k = divmod(name[2], 2)
            views = [((o_v, o_hbm), (slice(i * DH, (i + 1) * DH), slice(n * TM + k * FC, n * TM + (k + 1) * FC)))]
        return [pltpu.make_async_copy(src.at[idx], dst.at[idx], sems.at[sem_ids.setdefault((name, i), len(sem_ids))])
                for i, ((src, dst), idx) in enumerate(views)]

    def start(*names):
        for name in names:
            in_flight.append(name)
            for cp in copies(name):
                cp.start()

    def wait(*names):
        for name in names:
            in_flight.remove(name)
            for cp in copies(name):
                cp.wait()

    def prep_coefs():
        sk = sk_ref[...].astype(F32)
        for j in range(taps):
            coef[j] = jnp.broadcast_to(sk[j:j + 1], (LANES, D)).T
        coef[taps] = jnp.broadcast_to(d_ref[...].astype(F32).reshape(1, D), (LANES, D)).T

    first_pass, total_passes = {}, 0
    for r in range(7):
        first_pass[r] = total_passes
        total_passes += 3 if r in SHORT else 7

    k_tiles = ((0, 1), (2, 3), (4, 5), (6, 6), (2, 2))

    def wt_pieces(c):
        def piece(m, i, j):
            w = (wg_v, wu_v)[m]
            rows = jnp.concatenate([w[u * HALF:(u + 1) * HALF, tile(2 * c + i)] for u in k_tiles[j]], axis=0)
            wt[c, m, i, j] = pltpu.bitcast(rows.T, U32)

        return [part(piece, m, i, j) for m in range(2) for i in range(2) for j in range(len(k_tiles))]

    def wgu_pieces(c):
        def group(m, g, products):
            @functools.cache
            def raw(i, e, j):
                at = e * HALF // 2 + g * SUB
                return pltpu.bitcast(after(wt[c, m, i, j, at:at + SUB]), BF16).astype(F32)

            for r in products:
                piece(m, g, r, raw)

        def piece(m, g, r, raw):
            low = jax.lax.broadcasted_iota(jnp.int32, (2 * SUB, LANES), 1) < HALF

            def put(s, val):
                at = m * HALF // 16 + g
                wgu[c, first_pass[r] + s, at:at + 1] = _fold(val)

            if r in SHORT:
                head = [_combo(LHS_TERMS[r], lambda n: raw(n // 2, e, (0, 2)[n % 2])) for e in range(2)]
                tail = [_combo(LHS_TERMS[r], lambda n: raw(n // 2, e, (4, 3)[n % 2])) for e in range(2)]
                put(0, head[0] - jnp.where(low, 0.0, head[1]))
                put(1, jnp.where(low, head[1], tail[1] - tail[0]))
                put(2, jnp.where(low, tail[0], head[1]))
            else:
                def padded(e, a, n):
                    j = 2 * (n % 2) + a
                    return jnp.where(low, raw(n // 2, e, j), 0.0) if j == 3 else raw(n // 2, e, j)
                quads = [_combo(LHS_TERMS[r], part(padded, e, a)) for e in range(2) for a in range(2)]
                for s in range(7):
                    put(s, _combo(LHS_TERMS[s], quads.__getitem__))

        return [part(group, m, g, rs) for rs in opt.get("wg", ((2, 4, 5), (1, 3, 0, 6))) for m in range(2) for g in range(HALF // 16)]

    def wd_pieces():
        def rows(i, e, g):
            r0 = i * DH + e * DQ + 16 * g
            return slice(r0, r0 + 16)

        def paired(r, j, gs):
            half = after(jnp.full((1, LANES), 0.5, F32))
            for g in gs:
                def pick(e, n):
                    i, f = divmod(n, 2)
                    return jnp.stack(_zip_halves(wd_v[rows(i, e, g), tile(4 * j + f)], wd_v[rows(i, e, g), tile(4 * j + 2 + f)]))
                left = [half * _combo(LHS_TERMS[r], part(pick, e)) for e in range(2)]
                for s in range(7):
                    wd2[r, s, j, g:g + 1] = _fold(_combo(LHS_TERMS[s], lambda n: left[n // 2][n % 2]))

        def last(r):
            half = after(jnp.full((1, LANES), 0.5, F32))
            for e in range(2):
                for g in range(DQ // 16):
                    pick = lambda n: wd_v[rows(n // 2, e, g), tile(2 * NCH - 2 + n % 2)].astype(F32)
                    wd1[r, e, g:g + 1] = _fold(half * _combo(LHS_TERMS[r], pick))

        groups = np.array_split(np.arange(DQ // 16), opt.get('wd', 7))
        return {r: [part(paired, r, j, [int(g) for g in gs]) for j in range(NCH // 2) for gs in groups] + [part(last, r)]
                for r in range(7)}

    def kv_rows(j, r0, nr):
        rows = slice(r0, r0 + nr)
        lane = jax.lax.broadcasted_iota(jnp.int32, (SUB, LANES), 1)
        lane = jnp.concatenate([after(lane) if opt.get("chain", 1) else lane] * (nr // 16), axis=0)
        cur = pltpu.bitcast(k_v[rows, tile(j)], U32)
        prev = pltpu.bitcast(k_v[rows, tile(j - 1)], U32) if j > 0 else jnp.zeros_like(cur)
        ksh = pltpu.bitcast(cur, BF16).astype(F32) * coef[0, rows, :]
        for t in range(1, taps):
            moved = pltpu.roll(jnp.where(lane >= LANES - t, prev, cur), t, 1)
            ksh = ksh + pltpu.bitcast(moved, BF16).astype(F32) * coef[t, rows, :]
        kv_s[j, r0 // 16:(r0 + nr) // 16] = _fold(ksh * v_v[rows, tile(j)].astype(F32))

    def kv_pieces(b, halves=(0, 1)):
        return [part(kv_rows, 4 * b + n, i * DH + r0, 16) for i in halves for n in range(4) for r0 in range(0, DH, 16)]

    def fx(b, i):
        rows = slice(i * DH, (i + 1) * DH)
        prev = (hprev[0, rows, :], hprev[1, rows, :]) if b else None
        for j in range(4 * b, 4 * b + 4):
            hf = dot(lambda: h_v[rows, tile(j)], lambda: fwd_ref[...])
            hr, hi = hf[:, :LANES], hf[:, LANES:]
            if j == 0:
                hr = hr + coef[taps, rows, :]
            c, d = (hr + prev[1], hi - prev[0]) if prev else (hr, hi)
            prev = (hr, hi)
            spec[j, 0, rows, :], spec[j, 1, rows, :], spec[j, 2, rows, :] = c, d - c, c + d
        if b + 1 < NBLK:
            hprev[0, rows, :], hprev[1, rows, :] = prev
        for j in range(4 * b, 4 * b + 4):
            xf = dot(lambda: _unfold(kv_s[j, i * DH // 16:(i + 1) * DH // 16]), lambda: fwd_ref[...])
            a, s = xf[:, :LANES], xf[:, LANES:]
            spec[j, 3, rows, :], spec[j, 4, rows, :], spec[j, 5, rows, :] = a + s, a, s

    def conv_pieces(b, halves=(0, 1)):
        st = {}
        mode = opt.get("chain", 1)

        def plane(hi, r0, p):
            rows = slice(r0, r0 + SUB)
            newer = spec[hi, p, rows, :]
            acc = [None, None]

            def term(n, t):
                if acc[n] is not None:
                    acc[n] = acc[n] - t if p == 2 else acc[n] + t
                elif p == 0:
                    acc[n] = after(t) if mode else t
                else:
                    base = after(st[n]) if mode else st[n]
                    acc[n] = base + t if p == 1 else base - t

            for j in range(hi + 1):
                xv = spec[j, 3 + p, rows, :]
                term(1, newer * xv)
                if j < hi:
                    newer = spec[hi - 1 - j, p, rows, :]
                    term(0, newer * xv)
            for n in range(2):
                if p == 0:
                    st[n] = acc[n]
                else:
                    yf_s[hi - 1 + n, rows, tile(2 - p)] = acc[n].astype(BF16)

        def both(hi, r0):
            plane(hi, r0, 0)
            plane(hi, r0, 1)

        return [f for i in halves for hi in (4 * b + 1, 4 * b + 3) for r0 in range(i * DH, (i + 1) * DH, SUB)
                for f in ([part(plane, hi, r0, p) for p in range(3)] if mode else (part(both, hi, r0), part(plane, hi, r0, 2)))]

    def inv(b, i):
        rows = slice(i * DH, (i + 1) * DH)
        for j in range(4 * b, 4 * b + 4):
            y_s[rows, tile(j)] = dot(lambda: yf_s[j, rows, :], lambda: inv_ref[...])

    def pre_pieces(b, layer):
        st = {}
        rows_per = opt.get("pr", 64)
        keep = opt.get("keep", 1)

        def accumulate(t, r0, val):
            for i in range(0, val.shape[0], SUB):
                st["sum", t] = st["sum", t] + val[i:i + SUB] if r0 + i else val[:SUB]
            return jnp.sum(st["sum", t], axis=0, keepdims=True) * (1.0 / D) if r0 + rows_per == D else None

        def first(t, r0):
            idx = (slice(r0, r0 + rows_per), tile(4 * b + t))
            st["x", t, r0] = q_v[idx].astype(F32) if layer == 0 else x_s[idx]
            st["x", t, r0] = jnp.concatenate([after(st["x", t, r0][:SUB]), st["x", t, r0][SUB:]], axis=0)
            st["m", t] = accumulate(t, r0, st["x", t, r0])

        def rstd(t, r0):
            c = st["c", t, r0] = st["x", t, r0] - after(st["m", t])
            var = accumulate(t, r0, c * c)
            if var is not None:
                st["r", t] = jax.lax.rsqrt(var + EPS)

        def gate(t, r0):
            idx = (slice(r0, r0 + rows_per), tile(4 * b + t))
            if keep:
                normed = st["c", t, r0] * after(st["r", t])
            else:
                normed = (st["x", t, r0] - after(st["m", t])) * st["r", t]
            x = st["x", t, r0] = st["x", t, r0] + normed * y_s[idx]
            x_s[idx] = x
            mean = accumulate(t, r0, x)
            if mean is not None:
                st["m", t] = mean

        def combos(u, r0, products):
            scale = functools.cache(lambda t: after(st["r" if keep else "m", t]))
            at = (u * HALF + r0) // 16

            @functools.cache
            def normed(j, a, t):
                row = (4 * j + 2 * a + u) * HALF + r0
                if row >= D:
                    return None
                r1, off = row // rows_per * rows_per, row % rows_per
                if keep:
                    return st["c", t, r1][off:off + 16] * scale(t)
                return (st["x", t, r1][off:off + 16] - scale(t)) * st["r", t]

            for r in products:
                right = lambda a, t: _combo(RHS_TERMS[r], lambda n: normed(n // 2, a, 2 * (n % 2) + t))
                h0 = first_pass[r] + sum(x < r for x in SHORT)
                if r in SHORT:
                    for t in range(2):
                        for a in range(2 - u):
                            hc[0, h0 + 2 * t + a, at:at + 1] = _fold(right(a, t))
                else:
                    quads = [right(a, t) for a in range(2) for t in range(2)]
                    for s in range(7):
                        hc[0, h0 + s, at:at + 1] = _fold(_combo(RHS_TERMS[s], quads.__getitem__))

        groups = opt.get("groups", ((0,), (1, 3), (5,), (2,), (4, 6)))
        stats = [part(f, t, r0) for f in (first, rstd, gate, rstd) for t in range(4) for r0 in range(0, D, rows_per)]
        return stats, [part(combos, u, r0, g) for g in groups for u in range(2) for r0 in range(0, HALF, 16)]

    def spread_pre(b, layer, lo, hi):
        stats, combos = pre_pieces(b, layer)
        hi -= opt.get("lead", 20)
        mid = lo + int((hi - lo) * opt.get("mid", 0.68))
        spread(stats, lo, mid)
        spread(combos, mid, hi)

    def gu(b, layer, c):
        lhs = lambda p: _unfold(wgu[c, p])
        rhs = hc.at[0]

        def outer(r):
            p0 = first_pass[r]
            h0 = p0 + sum(x < r for x in SHORT)
            if r not in SHORT:
                return _inner_sum(lambda s: dot(part(lhs, p0 + s), lambda: _unfold(rhs[h0 + s])))
            out = [None] * 4
            for t in range(2):
                u0, u1, u2 = (lambda: rhs[h0 + 2 * t, 0:4]), (lambda: rhs[h0 + 2 * t, 4:8]), (lambda: rhs[h0 + 2 * t + 1, 0:4])
                both = dot(part(lhs, p0 + 2), lambda: _unfold(jnp.concatenate([u2(), u1()], axis=0)))
                out[t] = dot(part(lhs, p0), lambda: _unfold(rhs[h0 + 2 * t])) + both
                out[2 + t] = dot(part(lhs, p0 + 1), lambda: _unfold(jnp.concatenate([u0(), u2()], axis=0))) + both
            return out

        acts = {}
        _outer_sum(outer, OUTER_ORDER, lambda m, quad: acts.update({m: [_geglu2(v) for v in quad]}))
        for r in range(7):
            right = [_combo(RHS_TERMS[r], lambda m: acts[m ^ 1][n]) for n in range(4)]
            if c < NCH // 2 * 2:
                for s in range(7):
                    ac2[layer, r, s, 4 * c:4 * c + 4] = _fold(_combo(RHS_TERMS[s], right.__getitem__))
            else:
                for n in range(4):
                    ac1[layer, r, n % 2, 4 * (n // 2):4 * (n // 2) + 4] = _fold(right[n])

    def dn(b, layer):
        def outer(r):
            one = lambda s, j: dot(lambda: _unfold(wd2[r, s, j]), lambda: _unfold(ac2[layer, r, s, SUB * j:SUB * (j + 1)]))
            out = _inner_sum(lambda s: functools.reduce(jnp.add, [one(s, j) for j in range(NCH // 2)]))
            return [out[n] + dot(lambda: _unfold(wd1[r, n // 2]), lambda: _unfold(ac1[layer, r, n % 2]))
                    for n in range(4)]

        def emit(m, quad):
            for n, val in enumerate(quad):
                r0 = (m // 2) * DH + (n // 2) * DQ
                idx = (slice(r0, r0 + DQ), tile(4 * b + 2 * (1 - m % 2) + n % 2))
                if layer == 0:
                    x_s[idx] = x_s[idx] + val
                else:
                    o_v[idx] = (x_s[idx] + val).astype(BF16)

        _outer_sum(outer, DOWN_ORDER, emit)

    slots = {fx: 8, inv: 4, gu: 46, dn: 175}
    regions, begin, end, total = [[]], {}, {}, [0]

    def add(name, fn, *args):
        begin.setdefault(name, total[0])
        total[0] += slots[fn]
        end[name] = total[0]
        regions[-1].append(part(fn, *args))

    def add_gu(b, layer, chunks=None):
        for c in (range(NCH) if chunks is None else chunks):
            add(("gu", b, layer), gu, b, layer, c)
            begin["chunk", b, layer, c], end["chunk", b, layer, c] = total[0] - slots[gu], total[0]

    def add_halves(name, fn, b):
        for i in range(2):
            add((name, b), fn, b, i)

    def cut(*setup):
        if setup:
            regions.append(list(setup))
        regions.append([])

    def spread(pieces, lo, hi):
        assert lo < hi
        for n, piece in enumerate(pieces):
            pending.setdefault(lo + n * (hi - lo) // len(pieces), []).append(piece)

    def now(pieces):
        regions[-1].extend(pieces)

    def outs(b):
        return [("out", b, m) for m in range(4)]

    now([part(start, ("head", 0)), part(start, ("head", 1)), prep_coefs, part(wait, ("head", 0)), part(start, ("q", 0))])
    now(kv_pieces(0, [0]))
    add(("fx", 0), fx, 0, 0)
    now([part(wait, ("head", 1)), part(start, ("w", 0), ("w", 1))] + kv_pieces(0, [1]))
    add(("fx", 0), fx, 0, 1)
    now(conv_pieces(0, [0]))
    add(("inv", 0), inv, 0, 0)
    now(conv_pieces(0, [1]))
    add(("inv", 0), inv, 0, 1)
    now([part(wait, ("q", 0), ("w", 0)), part(start, ("w", 2), ("w", 3))] + wt_pieces(0) + sum(pre_pieces(0, 0), []) + wgu_pieces(0))
    now([part(wait, ("w", 1))] + wt_pieces(1))
    cuts = {0: ([("w", 2)], [("w", 4), ("w", 5)]),
            1: ([("w", 3), ("w", 4)], [("w", 6), ("conv", 1)]),
            3: ([("w", 5), ("w", 6)], [("wd", 0), ("q", 1)]),
            6: ([("conv", 1), ("wd", 0)], [("conv", 2)])}
    for c in range(NCH):
        if c in cuts:
            cut(part(wait, *cuts[c][0]), part(start, *cuts[c][1]))
        add_gu(0, 0, [c])
        spread(wgu_pieces(c + 1) if c + 1 < NCH else kv_pieces(1), begin["chunk", 0, 0, c], end["chunk", 0, 0, c] - 8)
        if c + 2 < NCH:
            spread(wt_pieces(c + 2), begin["chunk", 0, 0, c], end["chunk", 0, 0, c] - 8)

    def job(b, layer):
        add_gu(b, layer)
        add(("dn", b, layer), dn, b, layer)

    wd_prep = wd_pieces()
    add_halves("fx", fx, 1)
    spread(wd_prep[DOWN_ORDER[0]] + wd_prep[DOWN_ORDER[1]], begin["fx", 1], end["fx", 1])
    cut(part(wait, ("conv", 2), ("q", 1)))
    add(("dn", 0, 0), dn, 0, 0)
    lo = begin["dn", 0, 0]
    for n, r in enumerate(DOWN_ORDER[2:]):
        spread(wd_prep[r], lo + 25 * n, lo + 25 * (n + 1))
    spread(kv_pieces(2, [0]), lo + 100, lo + 160)
    spread(kv_pieces(2, [1]), lo + 140, end["dn", 0, 0])
    add_halves("fx", fx, 2)
    stats, combos = pre_pieces(0, 1)
    spread([p for p in stats if p.args[0] < 2], lo + 130, end["dn", 0, 0])
    spread([p for p in stats if p.args[0] >= 2], begin["fx", 2], begin["fx", 2] + 9)
    spread(combos, begin["fx", 2] + 9, end["fx", 2] - 2)
    add_gu(0, 1)
    spread(conv_pieces(1), begin["gu", 0, 1], end["gu", 0, 1] - 8)
    cut()
    add_halves("inv", inv, 1)
    add(("dn", 0, 1), dn, 0, 1)
    add_gu(1, 0)
    spread_pre(1, 0, end["inv", 1], end["dn", 0, 1])
    second = conv_pieces(2)
    split = int(len(second) * opt.get("c2", 0.3))
    spread(second[:split], begin["dn", 0, 1], end["dn", 0, 1])
    spread(second[split:], begin["gu", 1, 0], end["gu", 1, 0] - 8)
    spread([part(start, *outs(0))], begin["gu", 1, 0] + 8, begin["gu", 1, 0] + 9)
    add_halves("inv", inv, 2)
    add(("dn", 1, 0), dn, 1, 0)
    spread_pre(2, 0, end["inv", 2], end["dn", 1, 0])
    spread(kv_pieces(3), begin["dn", 1, 0], end["dn", 1, 0] - 14)
    add_halves("fx", fx, 3)
    cut()
    job(2, 0)
    add_gu(1, 1)
    spread_pre(1, 1, begin["dn", 2, 0], end["dn", 2, 0])
    third = conv_pieces(3)
    split = int(len(third) * opt.get("c3", 0.39))
    spread(third[:split], begin["gu", 2, 0], end["gu", 2, 0])
    spread(third[split:-split], begin["dn", 2, 0], end["dn", 2, 0])
    spread(third[-split:], begin["gu", 1, 1], end["gu", 1, 1] - 8)
    add_halves("inv", inv, 3)
    add(("dn", 1, 1), dn, 1, 1)
    spread_pre(3, 0, end["inv", 3], end["dn", 1, 1])
    if opt.get("cut3"):
        cut()
    job(3, 0)
    if opt.get("cut3"):
        cut()
    job(2, 1)
    job(3, 1)
    spread([part(start, *outs(1))], begin["gu", 3, 0] + 8, begin["gu", 3, 0] + 9)
    spread_pre(2, 1, begin["dn", 3, 0], end["dn", 3, 0])
    spread_pre(3, 1, begin["dn", 2, 1], end["dn", 2, 1])
    spread([part(start, *outs(2))], begin["gu", 3, 1] + 8, begin["gu", 3, 1] + 9)

    def tick(i, carry):
        marks[0] = i
        return carry

    only = opt.get("only")
    for n, region in enumerate(regions):
        if only is not None and n not in only:
            clock["slot"] += sum(slots.get(getattr(st, "func", None), 0) for st in region)
            continue
        if n:
            jax.lax.fori_loop(0, 2, tick, 0)
        clock.update(token=None, last=None, no_bits=None)
        with (jax.named_scope(f"R{n:02d}") if opt.get("scopes") else contextlib.nullcontext()):
            for stage in region:
                stage()
    if only is not None:
        print([(n, [getattr(getattr(st, "func", st), "__name__") for st in r][:3]) for n, r in enumerate(regions)])
        jax.lax.fori_loop(0, 2, tick, 0)
        for ref in (x_s, y_s):
            o_v[...] = ref[...].astype(BF16)
        o_v[0:8, 0:256] = wgu[1, 0, 0] + hc[0, 0, 0] + ac2[0, 0, 0, 0] + ac1[0, 0, 0, 0] + wd2[0, 0, 0, 0] + wd1[0, 0, 0] + kv_s[0, 0] + yf_s[0, 0:8]
        o_v[8:16, 0:128] = (spec[0, 0, 0:8] + pltpu.bitcast(wt[0, 0, 0, 0, 0:8], F32)).astype(BF16)
        start(*outs(0))
        wait(*outs(0))
    else:
        assert not pending
        start(*outs(NBLK - 1))
        wait(*[name for b in range(NBLK) for name in outs(b)])
        assert not in_flight


def make(flags=None, **opt):
    def run(A_q, A_k, A_v, A_shift_k, A_ssm_k, A_ssm_D, B_x, B_w_gate, B_w_up, B_w_down):
        _, S, D = A_q.shape
        F = B_w_gate.shape[1]
        taps = A_shift_k.shape[1]
        fwd, inv = _dft_tables()
        NCH, NB = F // FC, S // LANES
        hbm = pl.BlockSpec(memory_space=pltpu.HBM)
        vmem = pl.BlockSpec(memory_space=pltpu.VMEM)
        folded = lambda *lead: pltpu.VMEM(lead + (SUB, 2 * LANES), BF16)
        out = pl.pallas_call(
            functools.partial(_kernel, opt=opt),
            out_shape=jax.ShapeDtypeStruct((D, S), BF16),
            in_specs=[hbm, hbm, hbm, vmem, hbm, vmem, hbm, hbm, hbm, vmem, vmem],
            out_specs=hbm,
            scratch_shapes=[pltpu.VMEM((D, S), BF16)] * 4 + [pltpu.VMEM((D, F), BF16)] * 3 + [
                pltpu.VMEM((D, S), BF16),
                pltpu.VMEM((taps + 1, D, LANES), F32),
                pltpu.VMEM((NB, 6, D, LANES), F32),
                pltpu.VMEM((2, D, LANES), F32),
                folded(NB, D // 16),
                pltpu.VMEM((NB, D, 2 * LANES), BF16),
                pltpu.VMEM((D, S), F32),
                pltpu.VMEM((NCH, 2, 2, 5, HALF, LANES), U32),
                folded(NCH, 37, SUB),
                folded(7, 7, NCH // 2, D // 64),
                folded(7, 2, D // 64),
                pltpu.VMEM((D, S), F32),
                folded(1, 40, SUB),
                folded(2, 7, 7, NCH // 2 * SUB),
                folded(2, 7, 2, SUB),
                pltpu.SMEM((1,), jnp.int32),
                pltpu.SemaphoreType.DMA((48,)),
            ],
            compiler_params=pltpu.CompilerParams(vmem_limit_bytes=120 * 2**20, flags=flags),
        )(A_q[0].T, A_k[0].T, A_v[0].T, A_shift_k.T, A_ssm_k, A_ssm_D, B_w_gate, B_w_up, B_w_down.T, fwd, inv)
        return out.T[None]
    return run


@jax.jit
def pallas_interleave_layers__ssm_conv_h3__geglu_ffn__prompt_kernel(
        A_q, A_k, A_v, A_shift_k, A_ssm_k, A_ssm_D, B_x, B_w_gate, B_w_up, B_w_down):
    return make()(A_q, A_k, A_v, A_shift_k, A_ssm_k, A_ssm_D, B_x, B_w_gate, B_w_up, B_w_down)
```

```python
import functools

import jax
import jax.experimental.pallas as pl
import jax.experimental.pallas.tpu as pltpu
import jax.numpy as jnp
import numpy as np

F32, BF16, U32 = jnp.float32, jnp.bfloat16, jnp.uint32
LANES, HALF, SUB, PACKED = 128, 64, 8, 16
BLOCK = 4 * LANES
CHUNK = 2 * LANES
NUM_BLOCKS, NUM_CHUNKS = 4, 7
PAIRS = 2
EPS = 1e-5

GELU_SCALE = float((np.sqrt(2.0 / np.pi) * 0.044715) ** (1.0 / 3.0))
GELU_LINEAR = float(np.sqrt(2.0 / np.pi) / GELU_SCALE)
DOWN_SCALE = 0.5 / GELU_SCALE ** 2

LHS_TERMS = ((0, 1, 3), (2, 1, 3), (0, 0, 0), (3, 0, 0), (0, 1, 1), (2, -1, 0), (1, -1, 3))
RHS_TERMS = ((0, 1, 3), (0, 0, 0), (1, -1, 3), (2, -1, 0), (3, 0, 0), (0, 1, 1), (2, 1, 3))
OUT_TERMS = ({0: 1, 3: 1, 4: -1, 6: 1}, {2: 1, 4: 1}, {1: 1, 3: 1}, {0: 1, 1: -1, 2: 1, 5: 1})
GATE_UP_ORDER = (2, 4, 1, 3, 0, 6, 5)
DOWN_ORDER = (2, 4, 0, 1, 5, 3, 6)

SHORT = (3, 4, 6)
RHS_START = tuple(sum(4 if x in SHORT else 7 for x in range(r)) for r in range(8))
WEIGHT_TILES = ((0, 1), (2, 3), (4, 5), (6, 6), (2, 2))

GATE_UP_PASSES = sum(6 if r in SHORT else 7 for r in range(7))
DOWN_PASSES = 7 * PAIRS + 4 * (NUM_CHUNKS - 2 * PAIRS)


def _dft_tables():
    n = np.arange(LANES)[:, None]
    k = np.arange(LANES)[None, :]
    angle = np.pi * (((4 * k + 1) * n) % (4 * LANES)) / (2 * LANES)
    c, s = np.cos(angle), np.sin(angle)
    forward = np.concatenate([c, s], axis=1)
    inverse = np.concatenate([c.T, s.T], axis=0) / LANES
    return forward.astype(BF16), inverse.astype(BF16)


def _tile(j):
    return slice(j * LANES, (j + 1) * LANES)


def _combine(term, quadrant):
    a, sign, b = term
    a = quadrant(a)
    b = quadrant(b) if sign else None
    if b is None:
        return a
    if a is None:
        assert sign > 0
        return b
    return a + b if sign > 0 else a - b


def _inner_sum(product):
    m1, m2, m3, m4, m5, m6, m7 = (product(s) for s in range(7))
    return [(m1 + m4) - m5 + m7, m3 + m5, m2 + m4, (m1 - m2) + m3 + m6]


def _outer_sum(product, order, emit):
    m = {}
    for r in order:
        m[r] = product(r)
        for quadrant, terms in enumerate(OUT_TERMS):
            if r in terms and all(x in m for x in terms):
                names = sorted(terms, key=lambda x: (x != r, terms[x] < 0))
                if terms[names[0]] < 0:
                    names[0], names[1] = names[1], names[0]
                blocks = list(m[names[0]])
                for x in names[1:]:
                    blocks = [u + v if terms[x] > 0 else u - v for u, v in zip(blocks, m[x])]
                emit(quadrant, blocks)


def _fold(x):
    x = x.reshape(x.shape[0] // PACKED, 2, SUB, LANES)
    return jnp.concatenate([x[:, 0], x[:, 1]], axis=-1).astype(BF16)


def _unfold(v):
    return jnp.stack([v[:, :, :LANES], v[:, :, LANES:]], axis=1).reshape(PACKED * v.shape[0], LANES)


def _low_lanes(shape):
    return jax.lax.broadcasted_iota(jnp.int32, shape, 1) < HALF


def _zip_halves(a, b):
    a, b = pltpu.bitcast(a, U32), pltpu.bitcast(b, U32)
    low = _low_lanes(a.shape)
    swap = pltpu.roll(jnp.where(low, b, a), HALF, 1)
    return [pltpu.bitcast(v, BF16).astype(F32) for v in (jnp.where(low, a, swap), jnp.where(low, swap, b))]


def _geglu(gate_up):
    g, u = gate_up[:HALF], gate_up[HALF:]
    return (g * u) * (1.0 + jnp.tanh(g * (GELU_LINEAR + g * g)))


class _Schedule:
    def __init__(self, table_ref, mark_ref):
        self.table_ref, self.mark_ref = table_ref, mark_ref
        self.steps, self.room, self.pending = [], [], {}
        self.slot = 0
        self.reset()

    def reset(self):
        self.token = self.last = self._never = self._zero = None

    def unpin(self):
        self.token = self.last = None

    @property
    def planned(self):
        return len(self.room)

    def add(self, room, fn, *args):
        self.room.extend(room)
        self.steps.append(functools.partial(fn, *args))

    def now(self, *pieces):
        self.steps.extend(pieces)

    def cut(self, *transfers):
        if transfers:
            self.now(self._block_end, *transfers)
        self.now(self._block_end)

    def _block_end(self):
        def tick(i, carry):
            self.mark_ref[0] = i
            return carry

        jax.lax.fori_loop(0, 2, tick, 0)
        self.reset()

    def spread(self, pieces, lo, hi):
        weight = np.cumsum(self.room[lo:hi])
        for n, piece in enumerate(pieces):
            at = int(np.searchsorted(weight, (n + 0.5) / len(pieces) * weight[-1]))
            self.pending.setdefault(lo + at, []).append(piece)

    def after(self, x):
        if self.token is None:
            return x
        if self._never is None:
            self._never = self.table_ref[0:PACKED, :LANES].astype(F32)[:SUB] > 2.0
        token = self.token if self.token.dtype == x.dtype else pltpu.bitcast(self.token, x.dtype)
        return jnp.where(self._never[:x.shape[0]], token[:x.shape[0]], x)

    def zero(self):
        if self._zero is None:
            self._zero = (pltpu.bitcast(self.table_ref[0:PACKED, LANES:], jnp.int32)[0, 0] << 16) >> 16
        return self._zero

    def dot(self, lhs, rhs):
        pieces = self.pending.pop(self.slot, ())
        for n, piece in enumerate(pieces):
            if self.last is not None:
                regs = self.last.shape[0] // SUB
                if regs <= PACKED:
                    row = (self.slot % 4 * len(pieces) + n) * regs // (4 * len(pieces)) * SUB
                else:
                    row = n * regs // len(pieces) * SUB
                self.token = self.last[row:row + SUB, :LANES]
            piece()
        self.slot += 1
        self.last = jnp.dot(lhs(), rhs(), preferred_element_type=F32)
        return self.last

    def run(self):
        for step in self.steps:
            step()
        assert not self.pending


def _kernel(q_hbm, k_hbm, v_hbm, taps_hbm, h_hbm, skip_hbm, wg_hbm, wu_hbm, wd_hbm, fwd_hbm, inv_hbm,
            o_hbm,
            taps_v, skip_v, fwd_v, inv_v, q_v, k_v, v_v, h_v, wg_v, wu_v, wd_v, o_v,
            coef, spectra, h_prev, kv_s, y_freq, y_s, w_t, w_gu, wd_pair, wd_rest, x_s,
            h_ops, act_pair, act_rest, mark, sems):
    D = q_v.shape[0]
    DH, DQ = D // 2, D // 4
    taps = taps_v.shape[0]
    part = functools.partial
    plan = _Schedule(fwd_v, mark)
    dot, after = plan.dot, plan.after

    sem_ids, in_flight = {}, []

    def copies(name):
        kind, n = name[:2]
        every = slice(None)
        kv_pair = ((k_hbm, k_v), (v_hbm, v_v))
        if kind == "coefs":
            views = [(p, ...) for p in ((taps_hbm, taps_v), (skip_hbm, skip_v))]
        elif kind == "tables":
            views = [(p, ...) for p in ((fwd_hbm, fwd_v), (inv_hbm, inv_v))]
        elif kind == "kv0":
            views = [(p, (slice(n * DQ, (n + 1) * DQ), slice(0, BLOCK))) for p in kv_pair]
        elif kind == "h0":
            views = [((h_hbm, h_v), (slice(n * DH, (n + 1) * DH), slice(0, BLOCK)))]
        elif kind == "kv":
            cols = slice(BLOCK, 2 * BLOCK) if n == 1 else slice(2 * BLOCK, None)
            views = [(p, (every, cols)) for p in kv_pair]
        elif kind == "h":
            views = [((h_hbm, h_v), (every, slice(n * BLOCK, (n + 1) * BLOCK)))]
        elif kind == "q":
            views = [((q_hbm, q_v), (every, slice(0, BLOCK) if n == 0 else slice(BLOCK, None)))]
        elif kind == "w":
            views = [(p, (every, slice(n * CHUNK, (n + 1) * CHUNK))) for p in ((wg_hbm, wg_v), (wu_hbm, wu_v))]
        elif kind == "wd":
            views = [((wd_hbm, wd_v), (every, every))]
        else:
            i, k = divmod(name[2], 2)
            col = n * BLOCK + k * CHUNK
            views = [((o_v, o_hbm), (slice(i * DH, (i + 1) * DH), slice(col, col + CHUNK)))]
        return [pltpu.make_async_copy(src.at[idx], dst.at[idx], sems.at[sem_ids.setdefault((name, i), len(sem_ids))])
                for i, ((src, dst), idx) in enumerate(views)]

    def start(*names):
        for name in names:
            in_flight.append(name)
            for copy in copies(name):
                copy.start()

    def wait(*names):
        for name in names:
            in_flight.remove(name)
            for copy in copies(name):
                copy.wait()

    def outputs(b):
        return [("out", b, m) for m in range(4)]

    def broadcast_coefs():
        rows = taps_v[...].astype(F32)
        for j in range(taps):
            coef[j] = jnp.broadcast_to(rows[j:j + 1], (LANES, D)).T
        coef[taps] = jnp.broadcast_to(skip_v[...].astype(F32).reshape(1, D), (LANES, D)).T

    def transpose_pieces(c, pin=False):
        def piece(m, i):
            w = (wg_v, wu_v)[m]
            groups = [w[u * HALF:(u + 1) * HALF, _tile(2 * c + i)] for pair in WEIGHT_TILES for u in pair]
            words = pltpu.bitcast(jnp.concatenate(groups, axis=0).T, U32)
            for j in range(len(WEIGHT_TILES)):
                w_t[c][m, i, j] = words[:, _tile(j)]
            if pin:
                plan.token = words[:SUB, :LANES]

        return [part(piece, m, i) for m in range(2) for i in range(2)]

    def gate_up_weight_pieces(c, pin=False):
        def piece(m, g, products):
            @functools.cache
            def raw(i, e, j):
                at = e * HALF // 2 + g * SUB
                if pin:
                    words = after(w_t[c][m + plan.zero(), i, j, at:at + SUB])
                else:
                    words = w_t[c][m, i, j, at:at + SUB]
                return pltpu.bitcast(words, BF16).astype(F32)

            for r in products:
                low = _low_lanes((PACKED, LANES))
                at = m * HALF // PACKED + g

                def put(s, val):
                    w_gu[c][r][s, at:at + 1] = _fold(val)

                def padded(e, a, n):
                    j = 2 * (n % 2) + a
                    return jnp.where(low, raw(n // 2, e, j), 0.0) if j == 3 else raw(n // 2, e, j)

                if r in SHORT:
                    head = [_combine(LHS_TERMS[r], lambda n: raw(n // 2, e, (0, 2)[n % 2])) for e in range(2)]
                    tail = [_combine(LHS_TERMS[r], lambda n: raw(n // 2, e, (4, 3)[n % 2])) for e in range(2)]
                    put(0, head[0] - jnp.where(low, 0.0, head[1]))
                    put(1, jnp.where(low, head[1], tail[1] - tail[0]))
                    put(2, jnp.where(low, tail[0], head[1]))
                else:
                    quads = [_combine(LHS_TERMS[r], part(padded, e, a)) for e in range(2) for a in range(2)]
                    for s in range(7):
                        put(s, _combine(LHS_TERMS[s], quads.__getitem__))

        groups = range(HALF // PACKED)
        if pin:
            return [part(piece, m, g, rs) for m in range(2) for rs in ((2, 4), (1, 3), (0, 6), (5,)) for g in groups]
        return [part(piece, m, g, (r,)) for m in range(2) for g in groups for r in (0, 1, 3, 6, 5, 2, 4)]

    def down_weight_pieces(r):
        def rows(i, e, g):
            r0 = i * DH + e * DQ + PACKED * g
            return slice(r0, r0 + PACKED)

        def paired(j, g):
            scale = after(jnp.full((1, LANES), DOWN_SCALE, F32))

            def pick(e, n):
                i, f = divmod(n, 2)
                at = rows(i, e, g)
                return jnp.stack(_zip_halves(wd_v[at, _tile(4 * j + f)], wd_v[at, _tile(4 * j + 2 + f)]))

            left = [scale * _combine(LHS_TERMS[r], part(pick, e)) for e in range(2)]
            for s in range(7):
                wd_pair[r][s, j, g:g + 1] = _fold(_combine(LHS_TERMS[s], lambda n: left[n // 2][n % 2]))

        def single(c, e):
            scale = after(jnp.full((1, LANES), DOWN_SCALE, F32))
            for g in range(DQ // PACKED):
                pick = lambda n: wd_v[rows(n // 2, e, g), _tile(2 * c + n % 2)].astype(F32)
                wd_rest[r][c - 2 * PAIRS, e, g:g + 1] = _fold(scale * _combine(LHS_TERMS[r], pick))

        return ([part(paired, j, g) for j in range(PAIRS) for g in range(DQ // PACKED)]
                + [part(single, c, e) for e in range(2) for c in range(2 * PAIRS, NUM_CHUNKS)])

    def kv_pieces(b, halves=(0, 1)):
        def piece(j, r0):
            rows = slice(r0, r0 + PACKED)
            lane = after(jax.lax.broadcasted_iota(jnp.int32, (SUB, LANES), 1))
            cur = pltpu.bitcast(k_v[rows, _tile(j)], U32)
            prev = pltpu.bitcast(k_v[rows, _tile(j - 1)], U32) if j else jnp.zeros_like(cur)
            shifted = pltpu.bitcast(cur, BF16).astype(F32) * coef[0, rows, :]
            for t in range(1, taps):
                moved = pltpu.roll(jnp.where(lane >= LANES - t, prev, cur), t, 1)
                shifted = shifted + pltpu.bitcast(moved, BF16).astype(F32) * coef[t, rows, :]
            kv_s[j, r0 // PACKED:r0 // PACKED + 1] = _fold(shifted * v_v[rows, _tile(j)].astype(F32))

        return [part(piece, 4 * b + n, i * DH + r0) for i in halves for n in range(4) for r0 in range(0, DH, PACKED)]

    def filter_spectra(b, i):
        rows = slice(i * DH, (i + 1) * DH)
        prev = (h_prev[b - 1, 0, rows, :], h_prev[b - 1, 1, rows, :]) if b else None
        for j in range(4 * b, 4 * b + 4):
            freq = dot(lambda: h_v[rows, _tile(j)], lambda: fwd_v[...])
            re, im = freq[:, :LANES], freq[:, LANES:]
            if j == 0:
                re = re + coef[taps, rows, :]
            c, d = (re + prev[1], im - prev[0]) if prev else (re, im)
            prev = (re, im)
            spectra[j, 0, rows, :], spectra[j, 1, rows, :], spectra[j, 2, rows, :] = c, d - c, c + d
        if b + 1 < NUM_BLOCKS:
            h_prev[b, 0, rows, :], h_prev[b, 1, rows, :] = prev

    def signal_spectra(b, i):
        rows = slice(i * DH, (i + 1) * DH)
        for j in range(4 * b, 4 * b + 4):
            freq = dot(lambda: _unfold(kv_s[j, i * DH // PACKED:(i + 1) * DH // PACKED]), lambda: fwd_v[...])
            re, im = freq[:, :LANES], freq[:, LANES:]
            spectra[j, 3, rows, :], spectra[j, 4, rows, :], spectra[j, 5, rows, :] = re + im, re, im

    def conv_pieces(b, halves=(0, 1)):
        state = {}

        def plane(hi, r0, p, js):
            rows = slice(r0, r0 + SUB)
            for j in js:
                newer = state["h"] if j else spectra[hi, p, rows, :]
                signal = spectra[j, 3 + p, rows, :]
                terms = {1: newer * signal}
                if j < hi:
                    state["h"] = spectra[hi - 1 - j, p, rows, :]
                    terms[0] = state["h"] * signal
                for n, term in terms.items():
                    if j == 0 and p == 0:
                        state[n] = after(term)
                        continue
                    base = state["shared", n] if j == 0 else state[n]
                    base = after(base) if j == js[0] else base
                    state[n] = base - term if p == 2 else base + term
            if js[-1] == hi:
                for n in range(2):
                    if p == 0:
                        state["shared", n] = state[n]
                    else:
                        y_freq[hi - 1 + n, rows, _tile(2 - p)] = state[n].astype(BF16)

        runs = lambda hi: [range(hi + 1)] if hi < 8 else [range((hi + 1) // 2), range((hi + 1) // 2, hi + 1)]
        return [part(plane, hi, r0, p, js) for i in halves for hi in (4 * b + 1, 4 * b + 3)
                for r0 in range(i * DH, (i + 1) * DH, SUB) for p in range(3) for js in runs(hi)]

    def inverse(b, i):
        rows = slice(i * DH, (i + 1) * DH)
        for j in range(4 * b, 4 * b + 4):
            y_s[b][j % 4, rows, :] = dot(lambda: y_freq[j, rows, :], lambda: inv_v[...])

    def norm_pieces(b, layer):
        state = {}

        def fetch(stage, t, r0, size):
            if (b, layer) == (0, 0):
                return q_v[r0:r0 + size, _tile(t)].astype(F32) if stage < 3 else x_s[b][r0:r0 + size, _tile(t)]
            row = r0 + stage * plan.zero()
            if layer == 0 and stage < 3:
                return q_v[pl.ds(pl.multiple_of(row, PACKED), size), _tile(4 * b + t)].astype(F32)
            return x_s[b][pl.ds(pl.multiple_of(row, SUB), size), _tile(t)]

        def average(t, r0, val):
            for i in range(0, HALF, SUB):
                state["sum", t] = state["sum", t] + val[i:i + SUB] if r0 + i else val[:SUB]
            return jnp.sum(state["sum", t], axis=0, keepdims=True) * (1.0 / D) if r0 + HALF == D else None

        def center(t, r0):
            x = fetch(0, t, r0, HALF)
            state["mean", t] = average(t, r0, jnp.concatenate([after(x[:SUB]), x[SUB:]], axis=0))

        def deviation(stage, t, r0):
            centered = fetch(stage, t, r0, HALF) - after(state["mean", t])
            var = average(t, r0, centered * centered)
            if var is not None:
                state["scale", t] = jax.lax.rsqrt(var + EPS) * (GELU_SCALE if stage == 3 else 1.0)

        def gate(t, r0):
            rows = slice(r0, r0 + HALF)
            x = fetch(2, t, r0, HALF)
            x = x + (x - after(state["mean", t])) * state["scale", t] * y_s[b][t, rows, :]
            x_s[b][rows, _tile(t)] = x
            mean = average(t, r0, x)
            if mean is not None:
                state["mean", t] = mean

        def operands(u, r0, products):
            mean = functools.cache(lambda t: after(state["mean", t]))
            at = (u * HALF + r0) // PACKED

            @functools.cache
            def normed(j, a, t):
                row = (4 * j + 2 * a + u) * HALF + r0
                return (fetch(4 + products[0], t, row, PACKED) - mean(t)) * state["scale", t] if row < D else None

            for r in products:
                right = lambda a, t: _combine(RHS_TERMS[r], lambda n: normed(n // 2, a, 2 * (n % 2) + t))
                if r in SHORT:
                    for t in range(2):
                        for a in range(2 - u):
                            h_ops[RHS_START[r] + 2 * t + a, at:at + 1] = _fold(right(a, t))
                else:
                    quads = [right(a, t) for a in range(2) for t in range(2)]
                    for s in range(7):
                        h_ops[RHS_START[r] + s, at:at + 1] = _fold(_combine(RHS_TERMS[s], quads.__getitem__))

        stages = (center, part(deviation, 1), gate, part(deviation, 3))
        return ([part(stage, t, r0) for stage in stages for t in range(4) for r0 in range(0, D, HALF)],
                [part(operands, u, r0, rs) for rs in ((0,), (1, 3), (5,), (2,), (4, 6))
                 for u in range(2) for r0 in range(0, HALF, PACKED)])

    def gate_up(c, defer):
        def product(r):
            lhs = lambda s: lambda: _unfold(w_gu[c][r][s])
            at = RHS_START[r]
            if r not in SHORT:
                return _inner_sum(lambda s: dot(lhs(s), lambda: _unfold(h_ops[at + s])))
            out = [None] * 4
            for t in range(2):
                first, second = at + 2 * t, at + 2 * t + 1
                join = lambda a, b: _unfold(jnp.concatenate([a, b], axis=0))
                shared = dot(lhs(2), lambda: join(h_ops[second, 0:4], h_ops[first, 4:8]))
                out[t] = dot(lhs(0), lambda: _unfold(h_ops[first])) + shared
                out[2 + t] = dot(lhs(1), lambda: join(h_ops[first, 0:4], h_ops[second, 0:4])) + shared
            return out

        acts = {}
        _outer_sum(product, GATE_UP_ORDER, lambda m, blocks: acts.update({m: [_geglu(v) for v in blocks]}))

        def operands(r, g0, g1, late):
            def quadrant(n, m):
                x = acts[m ^ 1][n][PACKED * g0:PACKED * g1]
                if late and m == RHS_TERMS[r][0]:
                    x = jnp.concatenate([after(x[i:i + SUB]) for i in range(0, x.shape[0], SUB)], axis=0)
                return x

            right = [_combine(RHS_TERMS[r], part(quadrant, n)) for n in range(4)]
            if c < 2 * PAIRS:
                at = 4 * (c % 2)
                for s in range(7):
                    act_pair[c // 2][r, s, at + g0:at + g1] = _fold(_combine(RHS_TERMS[s], right.__getitem__))
            else:
                for n in range(4):
                    at = 4 * (n // 2)
                    act_rest[c - 2 * PAIRS][r, n % 2, at + g0:at + g1] = _fold(right[n])

        for r in range(7):
            if r not in defer:
                operands(r, 0, 4, False)
        if defer:
            plan.spread([part(operands, r, g, g + 1, True) for r in defer for g in range(4)],
                        plan.slot + 3, plan.slot + 11)

    def down(b, layer):
        def product(r):
            one = lambda s, j: dot(lambda: _unfold(wd_pair[r][s, j]), lambda: _unfold(act_pair[j][r, s]))
            out = _inner_sum(lambda s: functools.reduce(jnp.add, [one(s, j) for j in range(PAIRS)]))
            rest = lambda n, c: dot(lambda: _unfold(wd_rest[r][c, n // 2]), lambda: _unfold(act_rest[c][r, n % 2]))
            return [functools.reduce(jnp.add, [out[n]] + [rest(n, c) for c in range(len(act_rest))]) for n in range(4)]

        end = plan.slot + 7 * DOWN_PASSES

        def emit(m, blocks):
            for n, val in enumerate(blocks):
                r0 = (m // 2) * DH + (n // 2) * DQ
                rows, t = slice(r0, r0 + DQ), 2 * (1 - m % 2) + n % 2
                val = x_s[b][rows, _tile(t)] + val
                if layer == 0:
                    x_s[b][rows, _tile(t)] = val
                else:
                    o_v[rows, _tile(4 * b + t)] = val.astype(BF16)
            if layer == 1 and b == NUM_BLOCKS - 1:
                if plan.slot < end:
                    plan.pending.setdefault(plan.slot + 8, []).append(part(start, ("out", b, m ^ 1)))
                else:
                    start(("out", b, m ^ 1))

        _outer_sum(product, DOWN_ORDER, emit)

    gate_up_room = [0.1 if 9 <= i < 15 or 22 <= i < 28 or i >= 35 else 1.0 for i in range(GATE_UP_PASSES)]

    def add_gate_up(chunks=range(NUM_CHUNKS), defer=(3, 6)):
        lo = plan.planned
        for c in chunks:
            plan.add(gate_up_room, gate_up, c, defer if c + 1 < NUM_CHUNKS else ())
        return lo, plan.planned

    def add_down(b, layer):
        lo = plan.planned
        plan.add([1.0] * (7 * DOWN_PASSES), down, b, layer)
        return lo, plan.planned

    def add_transform(fn, b, halves=(0, 1)):
        lo = plan.planned
        for i in halves:
            plan.add([4.0] * 4, fn, b, i)
        return lo, plan.planned

    def spread_norm(b, layer, lo, hi):
        stats, ops = norm_pieces(b, layer)
        mid = lo + int((hi - lo) * 0.62)
        plan.spread(stats, lo, mid)
        plan.spread(ops, mid, hi)

    def send(b, job):
        plan.spread([part(start, *outputs(b))], job[0] + 8, job[0] + 9)

    plan.now(part(start, ("coefs", 0), ("tables", 0), ("h0", 0), ("kv0", 0), ("kv0", 1), ("h0", 1), ("kv0", 2),
                  ("kv0", 3), ("q", 0), ("h", 1), *[("w", c) for c in range(NUM_CHUNKS)], ("wd", 0), ("kv", 1),
                  ("h", 2), ("h", 3), ("kv", 2), ("q", 1)),
             part(wait, ("coefs", 0)), broadcast_coefs, part(wait, ("tables", 0), ("h0", 0)))
    add_transform(filter_spectra, 0, [0])
    plan.now(part(wait, ("kv0", 0), ("kv0", 1)), *kv_pieces(0, [0]))
    add_transform(signal_spectra, 0, [0])
    plan.cut(part(wait, ("h0", 1)))
    plan.spread(conv_pieces(0, [0]), *add_transform(filter_spectra, 0, [1]))
    plan.now(part(wait, ("kv0", 2), ("kv0", 3)), *kv_pieces(0, [1]))
    add_transform(signal_spectra, 0, [1])
    plan.cut()
    plan.spread(conv_pieces(0, [1]), *add_transform(inverse, 0, [0]))
    plan.now(part(wait, ("q", 0)))
    stats, ops = norm_pieces(0, 0)
    plan.spread(stats[:len(stats) // 2], *add_transform(inverse, 0, [1]))
    plan.cut(part(wait, ("h", 1)))
    plan.spread(stats[len(stats) // 2:], *add_transform(filter_spectra, 1))
    plan.now(part(wait, ("w", 0)), plan.unpin, *ops[:16])
    for n, piece in enumerate(transpose_pieces(0, pin=True)):
        plan.now(piece, *ops[16 + 6 * n:22 + 6 * n])
    plan.now(plan.unpin, *gate_up_weight_pieces(0))

    for c, arrivals in enumerate(((1,), (2, 3), (4,), (5,), (6,))):
        plan.cut(part(wait, *[("w", n) for n in arrivals]))
        lo, hi = add_gate_up([c], defer=())
        fresh = arrivals[0] == c + 1
        if fresh:
            plan.spread(transpose_pieces(c + 1), lo, lo + 2)
            lo += 5
        plan.spread(gate_up_weight_pieces(c + 1, pin=fresh), lo, hi - 1)
        plan.spread([piece for n in arrivals if n > c + 1 for piece in transpose_pieces(n)], lo, hi - 2)
    plan.cut(part(wait, ("wd", 0)))
    plan.spread(gate_up_weight_pieces(6), *add_gate_up([5], defer=()))
    lo, hi = add_gate_up([6])
    plan.spread([piece for r in DOWN_ORDER[:2] for piece in down_weight_pieces(r)], lo, hi - 1)
    plan.cut(part(wait, ("kv", 1), ("h", 2), ("h", 3)))
    lo, hi = add_down(0, 0)
    for n, r in enumerate(DOWN_ORDER[2:]):
        plan.spread(down_weight_pieces(r), lo + n * DOWN_PASSES, lo + (n + 1) * DOWN_PASSES)
    plan.spread(kv_pieces(1), lo + 2 * DOWN_PASSES, lo + 5 * DOWN_PASSES + 10)
    add_transform(filter_spectra, 2)
    add_transform(filter_spectra, 3)
    add_transform(signal_spectra, 1)
    stats, ops = norm_pieces(0, 1)
    plan.spread([piece for piece in stats if piece.args[-2] < 2], lo + 5 * DOWN_PASSES + 5, hi + 5)
    plan.spread([piece for piece in stats if piece.args[-2] >= 2], hi + 1, hi + 14)
    plan.spread(ops, hi + 14, plan.planned - 1)

    plan.cut(part(wait, ("kv", 2), ("q", 1)))
    lo, _ = add_gate_up()
    add_transform(signal_spectra, 2)
    plan.spread(kv_pieces(2), lo, lo + 2 * GATE_UP_PASSES)
    plan.spread(conv_pieces(1), lo + 2 * GATE_UP_PASSES, plan.planned)
    plan.cut()
    inv = add_transform(inverse, 1)
    _, hi = add_down(0, 1)
    spread_norm(1, 0, inv[1], hi - 12)
    conv = conv_pieces(2)
    split = len(conv) // 5 // 6 * 6
    plan.spread(conv[:split], inv[0], hi)

    plan.cut()
    job = add_gate_up()
    plan.spread(conv[split:], *job)
    send(0, job)
    plan.cut()
    inv = add_transform(inverse, 2)
    lo, hi = add_down(1, 0)
    add_transform(signal_spectra, 3)
    spread_norm(2, 0, inv[1], hi + 8)
    plan.spread(kv_pieces(3, [0]), inv[0], lo + 30)
    plan.spread(kv_pieces(3, [1]), lo + 30, hi)

    plan.cut()
    conv = conv_pieces(3)
    split = 2 * len(conv) // 5 // 6 * 6
    plan.spread(conv[:split], *add_gate_up())
    lo, hi = add_down(2, 0)
    spread_norm(1, 1, lo, hi - 12)
    plan.spread(conv[split:-split], lo, hi)
    plan.spread(conv[-split:], *add_gate_up())
    inv = add_transform(inverse, 3)
    _, hi = add_down(1, 1)
    spread_norm(3, 0, inv[1], hi - 12)

    plan.cut()
    send(1, add_gate_up())
    lo, hi = add_down(3, 0)
    spread_norm(2, 1, lo, hi - 12)
    add_gate_up()
    lo, hi = add_down(2, 1)
    spread_norm(3, 1, lo, hi - 12)
    plan.cut()
    send(2, add_gate_up())
    add_down(3, 1)
    plan.now(part(wait, *[name for b in range(NUM_BLOCKS) for name in outputs(b)]))

    plan.run()
    assert not in_flight


def _run(A_q, A_k, A_v, A_shift_k, A_ssm_k, A_ssm_D, B_x, B_w_gate, B_w_up, B_w_down):
    del B_x
    batch, S, D = A_q.shape
    F = B_w_gate.shape[1]
    taps = A_shift_k.shape[1]
    assert (batch, S, D, F) == (1, NUM_BLOCKS * BLOCK, 7 * HALF, NUM_CHUNKS * CHUNK)
    forward, inverse = _dft_tables()
    tiles, rest = S // LANES, NUM_CHUNKS - 2 * PAIRS
    hbm = pl.BlockSpec(memory_space=pltpu.HBM)
    folded = lambda *lead: pltpu.VMEM(lead + (SUB, 2 * LANES), BF16)
    out = pl.pallas_call(
        _kernel,
        out_shape=jax.ShapeDtypeStruct((D, S), BF16),
        in_specs=[hbm] * 11,
        out_specs=hbm,
        scratch_shapes=[
            *[pltpu.VMEM(shape, BF16) for shape in ((taps, D), (D,), forward.shape, inverse.shape)],
            *[pltpu.VMEM((D, S), BF16)] * 4,
            *[pltpu.VMEM((D, F), BF16)] * 3,
            pltpu.VMEM((D, S), BF16),
            pltpu.VMEM((taps + 1, D, LANES), F32),
            pltpu.VMEM((tiles, 6, D, LANES), F32),
            pltpu.VMEM((NUM_BLOCKS - 1, 2, D, LANES), F32),
            folded(tiles, D // PACKED),
            pltpu.VMEM((tiles, D, 2 * LANES), BF16),
            [pltpu.VMEM((4, D, LANES), F32)] * NUM_BLOCKS,
            [pltpu.VMEM((2, 2, len(WEIGHT_TILES), HALF, LANES), U32)] * NUM_CHUNKS,
            [[folded(3 if r in SHORT else 7, SUB) for r in range(7)]] * NUM_CHUNKS,
            [folded(7, PAIRS, D // 4 // PACKED)] * 7,
            [folded(rest, 2, D // 4 // PACKED)] * 7,
            [pltpu.VMEM((D, BLOCK), F32)] * NUM_BLOCKS,
            folded(RHS_START[7], SUB),
            [folded(7, 7, SUB)] * PAIRS,
            [folded(7, 2, SUB)] * rest,
            pltpu.SMEM((1,), jnp.int32),
            pltpu.SemaphoreType.DMA((56,)),
        ],
        compiler_params=pltpu.CompilerParams(
            vmem_limit_bytes=120 * 2**20, disable_bounds_checks=True, disable_semaphore_checks=True),
    )(A_q[0].T, A_k[0].T, A_v[0].T, A_shift_k.T, A_ssm_k, A_ssm_D, B_w_gate, B_w_up, B_w_down.T, forward, inverse)
    return out.T[None]


@jax.jit
def pallas_interleave_layers__ssm_conv_h3__geglu_ffn__prompt_kernel(
    A_q: jax.Array,
    A_k: jax.Array,
    A_v: jax.Array,
    A_shift_k: jax.Array,
    A_ssm_k: jax.Array,
    A_ssm_D: jax.Array,
    B_x: jax.Array,
    B_w_gate: jax.Array,
    B_w_up: jax.Array,
    B_w_down: jax.Array,
):
    return _run(A_q, A_k, A_v, A_shift_k, A_ssm_k, A_ssm_D, B_x, B_w_gate, B_w_up, B_w_down)
```

```python
import functools

import jax
import jax.experimental.pallas as pl
import jax.experimental.pallas.tpu as pltpu
import jax.numpy as jnp
import numpy as np

F32, BF16, U32 = jnp.float32, jnp.bfloat16, jnp.uint32
LANES, HALF, SUB, PACKED = 128, 64, 8, 16
BLOCK = 4 * LANES
CHUNK = 2 * LANES
NUM_BLOCKS, NUM_CHUNKS = 4, 7
PAIRS = 2
EPS = 1e-5

GELU_SCALE = float((np.sqrt(2.0 / np.pi) * 0.044715) ** (1.0 / 3.0))
GELU_LINEAR = float(np.sqrt(2.0 / np.pi) / GELU_SCALE)
DOWN_SCALE = 0.5 / GELU_SCALE ** 2

LHS_TERMS = ((0, 1, 3), (2, 1, 3), (0, 0, 0), (3, 0, 0), (0, 1, 1), (2, -1, 0), (1, -1, 3))
RHS_TERMS = ((0, 1, 3), (0, 0, 0), (1, -1, 3), (2, -1, 0), (3, 0, 0), (0, 1, 1), (2, 1, 3))
OUT_TERMS = ({0: 1, 3: 1, 4: -1, 6: 1}, {2: 1, 4: 1}, {1: 1, 3: 1}, {0: 1, 1: -1, 2: 1, 5: 1})
GATE_UP_ORDER = (2, 4, 1, 3, 0, 6, 5)
DOWN_ORDER = (2, 4, 0, 1, 5, 3, 6)

SHORT = (3, 4, 6)
RHS_START = tuple(sum(4 if x in SHORT else 7 for x in range(r)) for r in range(8))
WEIGHT_TILES = ((0, 1), (2, 3), (4, 5), (6, 6), (2, 2))

GATE_UP_PASSES = sum(6 if r in SHORT else 7 for r in range(7))
DOWN_PASSES = 7 * PAIRS + 4 * (NUM_CHUNKS - 2 * PAIRS)


def _tile(j):
    return slice(j * LANES, (j + 1) * LANES)


def _combine(term, quadrant):
    a, sign, b = term
    a = quadrant(a)
    b = quadrant(b) if sign else None
    if b is None:
        return a
    if a is None:
        assert sign > 0
        return b
    return a + b if sign > 0 else a - b


def _inner_sum(product):
    m1, m2, m3, m4, m5, m6, m7 = (product(s) for s in range(7))
    return [(m1 + m4) - m5 + m7, m3 + m5, m2 + m4, (m1 - m2) + m3 + m6]


def _outer_sum(product, order, emit):
    m = {}
    for r in order:
        m[r] = product(r)
        for quadrant, terms in enumerate(OUT_TERMS):
            if r in terms and all(x in m for x in terms):
                names = sorted(terms, key=lambda x: (x != r, terms[x] < 0))
                if terms[names[0]] < 0:
                    names[0], names[1] = names[1], names[0]
                blocks = list(m[names[0]])
                for x in names[1:]:
                    blocks = [u + v if terms[x] > 0 else u - v for u, v in zip(blocks, m[x])]
                emit(quadrant, blocks)


def _fold(x):
    x = x.reshape(x.shape[0] // PACKED, 2, SUB, LANES)
    return jnp.concatenate([x[:, 0], x[:, 1]], axis=-1).astype(BF16)


def _unfold(v):
    return jnp.stack([v[:, :, :LANES], v[:, :, LANES:]], axis=1).reshape(PACKED * v.shape[0], LANES)


def _low_lanes(shape):
    return jax.lax.broadcasted_iota(jnp.int32, shape, 1) < HALF


def _zip_halves(a, b):
    a, b = pltpu.bitcast(a, U32), pltpu.bitcast(b, U32)
    low = _low_lanes(a.shape)
    swap = pltpu.roll(jnp.where(low, b, a), HALF, 1)
    return [pltpu.bitcast(v, BF16).astype(F32) for v in (jnp.where(low, a, swap), jnp.where(low, swap, b))]


def _geglu(gate_up):
    g, u = gate_up[:HALF], gate_up[HALF:]
    return (g * u) * (1.0 + jnp.tanh(g * (GELU_LINEAR + g * g)))


class _Schedule:
    def __init__(self, table_ref, mark_ref):
        self.table_ref, self.mark_ref = table_ref, mark_ref
        self.steps, self.room, self.pending = [], [], {}
        self.slot = 0
        self.reset()

    def reset(self):
        self.token = self.last = self._never = self._zero = None

    def unpin(self):
        self.token = self.last = None

    @property
    def planned(self):
        return len(self.room)

    def add(self, room, fn, *args):
        self.room.extend(room)
        self.steps.append(functools.partial(fn, *args))

    def now(self, *pieces):
        self.steps.extend(pieces)

    def cut(self, *transfers):
        if transfers:
            self.now(self._block_end, *transfers)
        self.now(self._block_end)

    def _block_end(self):
        def tick(i, carry):
            self.mark_ref[0] = i
            return carry

        jax.lax.fori_loop(0, 2, tick, 0)
        self.reset()

    def spread(self, pieces, lo, hi):
        weight = np.cumsum(self.room[lo:hi])
        for n, piece in enumerate(pieces):
            at = int(np.searchsorted(weight, (n + 0.5) / len(pieces) * weight[-1]))
            self.pending.setdefault(lo + at, []).append(piece)

    def never(self):
        if self._never is None:
            self._never = self.table_ref[0:PACKED, :LANES].astype(F32)[:SUB] > 2.0
        return self._never

    def after(self, x):
        if self.token is None:
            return x
        token = self.token if self.token.dtype == x.dtype else pltpu.bitcast(self.token, x.dtype)
        return jnp.where(self.never()[:x.shape[0]], token[:x.shape[0]], x)

    def zero(self):
        if self._zero is None:
            self._zero = jnp.where(self.never(), SUB, 0)[0, 0]
        return self._zero

    def dot(self, lhs, rhs):
        pieces = self.pending.pop(self.slot, ())
        for n, piece in enumerate(pieces):
            if self.last is not None:
                regs = self.last.shape[0] // SUB
                if regs <= PACKED:
                    row = (self.slot % 4 * len(pieces) + n) * regs // (4 * len(pieces)) * SUB
                else:
                    row = n * regs // len(pieces) * SUB
                self.token = self.last[row:row + SUB, :LANES]
            piece()
        self.slot += 1
        self.last = jnp.dot(lhs(), rhs(), preferred_element_type=F32)
        return self.last

    def run(self):
        for step in self.steps:
            step()
        assert not self.pending


def _kernel(q_hbm, k_hbm, v_hbm, taps_hbm, h_hbm, skip_hbm, wg_hbm, wu_hbm, wd_hbm,
            o_hbm,
            taps_v, skip_v, fwd_v, inv_v, q_v, k_v, v_v, h_v, wg_v, wu_v, wd_v, o_v,
            coef, spectra, h_prev, kv_s, y_freq, y_s, w_t, w_gu, wd_pair, wd_rest, x_s,
            h_ops, act_pair, act_rest, mark, sems):
    D = q_v.shape[0]
    DH, DQ = D // 2, D // 4
    taps = taps_v.shape[0]
    part = functools.partial
    plan = _Schedule(fwd_v, mark)
    dot, after = plan.dot, plan.after

    sem_ids, in_flight = {}, []

    def copies(name):
        kind, n = name[:2]
        every = slice(None)
        kv_pair = ((k_hbm, k_v), (v_hbm, v_v))
        if kind == "coefs":
            views = [(p, ...) for p in ((taps_hbm, taps_v), (skip_hbm, skip_v))]
        elif kind == "kv0":
            views = [(p, (slice(n * DQ, (n + 1) * DQ), slice(0, BLOCK))) for p in kv_pair]
        elif kind == "h0":
            views = [((h_hbm, h_v), (slice(n * DH, (n + 1) * DH), slice(0, BLOCK)))]
        elif kind == "kv":
            cols = slice(BLOCK, 2 * BLOCK) if n == 1 else slice(2 * BLOCK, None)
            views = [(p, (every, cols)) for p in kv_pair]
        elif kind == "h":
            views = [((h_hbm, h_v), (every, slice(n * BLOCK, (n + 1) * BLOCK)))]
        elif kind == "q":
            views = [((q_hbm, q_v), (every, slice(0, BLOCK) if n == 0 else slice(BLOCK, None)))]
        elif kind == "w":
            views = [(p, (every, slice(n * CHUNK, (n + 1) * CHUNK))) for p in ((wg_hbm, wg_v), (wu_hbm, wu_v))]
        elif kind == "wd":
            views = [((wd_hbm, wd_v), (every, every))]
        else:
            i, k = divmod(name[2], 2)
            col = n * BLOCK + k * CHUNK
            views = [((o_v, o_hbm), (slice(i * DH, (i + 1) * DH), slice(col, col + CHUNK)))]
        return [pltpu.make_async_copy(src.at[idx], dst.at[idx], sems.at[sem_ids.setdefault((name, i), len(sem_ids))])
                for i, ((src, dst), idx) in enumerate(views)]

    def start(*names):
        for name in names:
            in_flight.append(name)
            for copy in copies(name):
                copy.start()

    def wait(*names):
        for name in names:
            in_flight.remove(name)
            for copy in copies(name):
                copy.wait()

    def outputs(b):
        return [("out", b, m) for m in range(4)]

    def broadcast_coefs():
        rows = taps_v[...].astype(F32)
        for j in range(taps):
            coef[j] = jnp.broadcast_to(rows[j:j + 1], (LANES, D)).T
        coef[taps] = jnp.broadcast_to(skip_v[...].astype(F32).reshape(1, D), (LANES, D)).T

    def forward_table():
        n = jax.lax.broadcasted_iota(jnp.int32, (LANES, LANES), 0)
        k = jax.lax.broadcasted_iota(jnp.int32, (LANES, LANES), 1)
        angle = (((4 * k + 1) * n) & (4 * LANES - 1)).astype(F32) * (np.pi / (2 * LANES))
        fwd_v[:, :LANES] = jnp.cos(angle).astype(BF16)
        fwd_v[:, LANES:] = jnp.sin(angle).astype(BF16)

    def inverse_table():
        inv_v[...] = (fwd_v[...].astype(F32).T * (1.0 / LANES)).astype(BF16)

    def transpose_pieces(c, pin=False):
        def piece(m, i):
            w = (wg_v, wu_v)[m]
            groups = [w[u * HALF:(u + 1) * HALF, _tile(2 * c + i)] for pair in WEIGHT_TILES for u in pair]
            words = pltpu.bitcast(jnp.concatenate(groups, axis=0).T, U32)
            for j in range(len(WEIGHT_TILES)):
                w_t[c][m, i, j] = words[:, _tile(j)]
            if pin:
                plan.token = words[:SUB, :LANES]

        return [part(piece, m, i) for m in range(2) for i in range(2)]

    def gate_up_weight_pieces(c, pin=False):
        def piece(m, g, products):
            @functools.cache
            def raw(i, e, j):
                at = e * HALF // 2 + g * SUB
                if pin:
                    words = after(w_t[c][m, i, j, pl.ds(pl.multiple_of(at + plan.zero(), SUB), SUB)])
                else:
                    words = w_t[c][m, i, j, at:at + SUB]
                return pltpu.bitcast(words, BF16).astype(F32)

            for r in products:
                low = _low_lanes((PACKED, LANES))
                at = m * HALF // PACKED + g

                def put(s, val):
                    w_gu[c][r][s, at:at + 1] = _fold(val)

                def padded(e, a, n):
                    j = 2 * (n % 2) + a
                    return jnp.where(low, raw(n // 2, e, j), 0.0) if j == 3 else raw(n // 2, e, j)

                if r in SHORT:
                    head = [_combine(LHS_TERMS[r], lambda n: raw(n // 2, e, (0, 2)[n % 2])) for e in range(2)]
                    tail = [_combine(LHS_TERMS[r], lambda n: raw(n // 2, e, (4, 3)[n % 2])) for e in range(2)]
                    put(0, head[0] - jnp.where(low, 0.0, head[1]))
                    put(1, jnp.where(low, head[1], tail[1] - tail[0]))
                    put(2, jnp.where(low, tail[0], head[1]))
                else:
                    quads = [_combine(LHS_TERMS[r], part(padded, e, a)) for e in range(2) for a in range(2)]
                    for s in range(7):
                        put(s, _combine(LHS_TERMS[s], quads.__getitem__))

        groups = range(HALF // PACKED)
        if pin:
            return [part(piece, m, g, rs) for m in range(2) for rs in ((2, 4), (1, 3), (0, 6), (5,)) for g in groups]
        return [part(piece, m, g, (r,)) for m in range(2) for g in groups for r in (0, 1, 3, 6, 5, 2, 4)]

    def down_weight_pieces(r):
        def rows(i, e, g):
            r0 = i * DH + e * DQ + PACKED * g
            return slice(r0, r0 + PACKED)

        def paired(j, g):
            scale = after(jnp.full((1, LANES), DOWN_SCALE, F32))

            def pick(e, n):
                i, f = divmod(n, 2)
                at = rows(i, e, g)
                return jnp.stack(_zip_halves(wd_v[at, _tile(4 * j + f)], wd_v[at, _tile(4 * j + 2 + f)]))

            left = [scale * _combine(LHS_TERMS[r], part(pick, e)) for e in range(2)]
            for s in range(7):
                wd_pair[r][s, j, g:g + 1] = _fold(_combine(LHS_TERMS[s], lambda n: left[n // 2][n % 2]))

        def single(c, e):
            scale = after(jnp.full((1, LANES), DOWN_SCALE, F32))
            for g in range(DQ // PACKED):
                pick = lambda n: wd_v[rows(n // 2, e, g), _tile(2 * c + n % 2)].astype(F32)
                wd_rest[r][c - 2 * PAIRS, e, g:g + 1] = _fold(scale * _combine(LHS_TERMS[r], pick))

        return ([part(paired, j, g) for j in range(PAIRS) for g in range(DQ // PACKED)]
                + [part(single, c, e) for e in range(2) for c in range(2 * PAIRS, NUM_CHUNKS)])

    def kv_pieces(b, halves=(0, 1)):
        def piece(j, r0):
            rows = slice(r0, r0 + PACKED)
            lane = after(jax.lax.broadcasted_iota(jnp.int32, (SUB, LANES), 1))
            cur = pltpu.bitcast(k_v[rows, _tile(j)], U32)
            prev = pltpu.bitcast(k_v[rows, _tile(j - 1)], U32) if j else jnp.zeros_like(cur)
            shifted = pltpu.bitcast(cur, BF16).astype(F32) * coef[0, rows, :]
            for t in range(1, taps):
                moved = pltpu.roll(jnp.where(lane >= LANES - t, prev, cur), t, 1)
                shifted = shifted + pltpu.bitcast(moved, BF16).astype(F32) * coef[t, rows, :]
            kv_s[j, r0 // PACKED:r0 // PACKED + 1] = _fold(shifted * v_v[rows, _tile(j)].astype(F32))

        return [part(piece, 4 * b + n, i * DH + r0) for i in halves for n in range(4) for r0 in range(0, DH, PACKED)]

    def filter_spectra(b, i):
        rows = slice(i * DH, (i + 1) * DH)
        prev = (h_prev[b - 1, 0, rows, :], h_prev[b - 1, 1, rows, :]) if b else None
        for j in range(4 * b, 4 * b + 4):
            freq = dot(lambda: h_v[rows, _tile(j)], lambda: fwd_v[...])
            re, im = freq[:, :LANES], freq[:, LANES:]
            if j == 0:
                re = re + coef[taps, rows, :]
            c, d = (re + prev[1], im - prev[0]) if prev else (re, im)
            prev = (re, im)
            spectra[j, 0, rows, :], spectra[j, 1, rows, :], spectra[j, 2, rows, :] = c, d - c, c + d
        if b + 1 < NUM_BLOCKS:
            h_prev[b, 0, rows, :], h_prev[b, 1, rows, :] = prev

    def signal_spectra(b, i):
        rows = slice(i * DH, (i + 1) * DH)
        for j in range(4 * b, 4 * b + 4):
            freq = dot(lambda: _unfold(kv_s[j, i * DH // PACKED:(i + 1) * DH // PACKED]), lambda: fwd_v[...])
            re, im = freq[:, :LANES], freq[:, LANES:]
            spectra[j, 3, rows, :], spectra[j, 4, rows, :], spectra[j, 5, rows, :] = re + im, re, im

    def conv_pieces(b, halves=(0, 1)):
        state = {}

        def plane(hi, r0, p, js):
            rows = slice(r0, r0 + SUB)
            for j in js:
                newer = state["h"] if j else spectra[hi, p, rows, :]
                signal = spectra[j, 3 + p, rows, :]
                terms = {1: newer * signal}
                if j < hi:
                    state["h"] = spectra[hi - 1 - j, p, rows, :]
                    terms[0] = state["h"] * signal
                for n, term in terms.items():
                    if j == 0 and p == 0:
                        state[n] = after(term)
                        continue
                    base = state["shared", n] if j == 0 else state[n]
                    base = after(base) if j == js[0] else base
                    state[n] = base - term if p == 2 else base + term
            if js[-1] == hi:
                for n in range(2):
                    if p == 0:
                        state["shared", n] = state[n]
                    else:
                        y_freq[hi - 1 + n, rows, _tile(2 - p)] = state[n].astype(BF16)

        runs = lambda hi: [range(hi + 1)] if hi < 8 else [range((hi + 1) // 2), range((hi + 1) // 2, hi + 1)]
        return [part(plane, hi, r0, p, js) for i in halves for hi in (4 * b + 1, 4 * b + 3)
                for r0 in range(i * DH, (i + 1) * DH, SUB) for p in range(3) for js in runs(hi)]

    def inverse(b, i):
        rows = slice(i * DH, (i + 1) * DH)
        for j in range(4 * b, 4 * b + 4):
            y_s[b][j % 4, rows, :] = dot(lambda: y_freq[j, rows, :], lambda: inv_v[...])

    def norm_pieces(b, layer):
        state = {}

        def fetch(stage, t, r0, size):
            if layer == 0 and stage < 3:
                return q_v[r0:r0 + size, _tile(4 * b + t)].astype(F32)
            if (b, layer) == (0, 0):
                return x_s[b][r0:r0 + size, _tile(t)]
            return x_s[b][pl.ds(pl.multiple_of(r0 + stage * plan.zero(), SUB), size), _tile(t)]

        def average(t, r0, val):
            for i in range(0, HALF, SUB):
                state["sum", t] = state["sum", t] + val[i:i + SUB] if r0 + i else val[:SUB]
            return jnp.sum(state["sum", t], axis=0, keepdims=True) * (1.0 / D) if r0 + HALF == D else None

        def center(t, r0):
            x = fetch(0, t, r0, HALF)
            state["mean", t] = average(t, r0, jnp.concatenate([after(x[:SUB]), x[SUB:]], axis=0))

        def deviation(stage, t, r0):
            centered = fetch(stage, t, r0, HALF) - after(state["mean", t])
            var = average(t, r0, centered * centered)
            if var is not None:
                state["scale", t] = jax.lax.rsqrt(var + EPS) * (GELU_SCALE if stage == 3 else 1.0)

        def gate(t, r0):
            rows = slice(r0, r0 + HALF)
            x = fetch(2, t, r0, HALF)
            x = x + (x - after(state["mean", t])) * state["scale", t] * y_s[b][t, rows, :]
            x_s[b][rows, _tile(t)] = x
            mean = average(t, r0, x)
            if mean is not None:
                state["mean", t] = mean

        def operands(u, r0, products):
            mean = functools.cache(lambda t: after(state["mean", t]))
            at = (u * HALF + r0) // PACKED

            @functools.cache
            def normed(j, a, t):
                row = (4 * j + 2 * a + u) * HALF + r0
                return (fetch(4 + products[0], t, row, PACKED) - mean(t)) * state["scale", t] if row < D else None

            for r in products:
                right = lambda a, t: _combine(RHS_TERMS[r], lambda n: normed(n // 2, a, 2 * (n % 2) + t))
                if r in SHORT:
                    for t in range(2):
                        for a in range(2 - u):
                            h_ops[RHS_START[r] + 2 * t + a, at:at + 1] = _fold(right(a, t))
                else:
                    quads = [right(a, t) for a in range(2) for t in range(2)]
                    for s in range(7):
                        h_ops[RHS_START[r] + s, at:at + 1] = _fold(_combine(RHS_TERMS[s], quads.__getitem__))

        stages = (center, part(deviation, 1), gate, part(deviation, 3))
        return ([part(stage, t, r0) for stage in stages for t in range(4) for r0 in range(0, D, HALF)],
                [part(operands, u, r0, rs) for rs in ((0,), (1, 3), (5,), (2,), (4, 6))
                 for u in range(2) for r0 in range(0, HALF, PACKED)])

    def gate_up(c, defer):
        def product(r):
            lhs = lambda s: lambda: _unfold(w_gu[c][r][s])
            at = RHS_START[r]
            if r not in SHORT:
                return _inner_sum(lambda s: dot(lhs(s), lambda: _unfold(h_ops[at + s])))
            out = [None] * 4
            for t in range(2):
                first, second = at + 2 * t, at + 2 * t + 1
                join = lambda a, b: _unfold(jnp.concatenate([a, b], axis=0))
                shared = dot(lhs(2), lambda: join(h_ops[second, 0:4], h_ops[first, 4:8]))
                out[t] = dot(lhs(0), lambda: _unfold(h_ops[first])) + shared
                out[2 + t] = dot(lhs(1), lambda: join(h_ops[first, 0:4], h_ops[second, 0:4])) + shared
            return out

        acts = {}
        _outer_sum(product, GATE_UP_ORDER, lambda m, blocks: acts.update({m: [_geglu(v) for v in blocks]}))

        def operands(r, g0, g1, late):
            def quadrant(n, m):
                x = acts[m ^ 1][n][PACKED * g0:PACKED * g1]
                if late and m == RHS_TERMS[r][0]:
                    x = jnp.concatenate([after(x[i:i + SUB]) for i in range(0, x.shape[0], SUB)], axis=0)
                return x

            right = [_combine(RHS_TERMS[r], part(quadrant, n)) for n in range(4)]
            if c < 2 * PAIRS:
                at = 4 * (c % 2)
                for s in range(7):
                    act_pair[c // 2][r, s, at + g0:at + g1] = _fold(_combine(RHS_TERMS[s], right.__getitem__))
            else:
                for n in range(4):
                    at = 4 * (n // 2)
                    act_rest[c - 2 * PAIRS][r, n % 2, at + g0:at + g1] = _fold(right[n])

        for r in range(7):
            if r not in defer:
                operands(r, 0, 4, False)
        if defer:
            plan.spread([part(operands, r, g, g + 1, True) for r in defer for g in range(4)],
                        plan.slot + 3, plan.slot + 11)

    def down(b, layer):
        def product(r):
            one = lambda s, j: dot(lambda: _unfold(wd_pair[r][s, j]), lambda: _unfold(act_pair[j][r, s]))
            out = _inner_sum(lambda s: functools.reduce(jnp.add, [one(s, j) for j in range(PAIRS)]))
            rest = lambda n, c: dot(lambda: _unfold(wd_rest[r][c, n // 2]), lambda: _unfold(act_rest[c][r, n % 2]))
            return [functools.reduce(jnp.add, [out[n]] + [rest(n, c) for c in range(len(act_rest))]) for n in range(4)]

        end = plan.slot + 7 * DOWN_PASSES

        def emit(m, blocks):
            for n, val in enumerate(blocks):
                r0 = (m // 2) * DH + (n // 2) * DQ
                rows, t = slice(r0, r0 + DQ), 2 * (1 - m % 2) + n % 2
                val = x_s[b][rows, _tile(t)] + val
                if layer == 0:
                    x_s[b][rows, _tile(t)] = val
                else:
                    o_v[rows, _tile(4 * b + t)] = val.astype(BF16)
            if layer == 1 and b == NUM_BLOCKS - 1:
                if plan.slot < end:
                    plan.pending.setdefault(plan.slot + 8, []).append(part(start, ("out", b, m ^ 1)))
                else:
                    start(("out", b, m ^ 1))

        _outer_sum(product, DOWN_ORDER, emit)

    def add_gate_up(chunks=range(NUM_CHUNKS), busy=0.1):
        lo = plan.planned
        room = [busy if 9 <= i < 15 or 22 <= i < 28 or i >= 35 else 1.0 for i in range(GATE_UP_PASSES)]
        for c in chunks:
            plan.add(room, gate_up, c, () if c + 1 == NUM_CHUNKS else (3, 6))
        return lo, plan.planned

    def add_down(b, layer):
        lo = plan.planned
        plan.add([1.0] * (7 * DOWN_PASSES), down, b, layer)
        return lo, plan.planned

    def add_transform(fn, b, halves=(0, 1)):
        lo = plan.planned
        for i in halves:
            plan.add([4.0] * 4, fn, b, i)
        return lo, plan.planned

    def spread_norm(b, layer, lo, hi):
        stats, ops = norm_pieces(b, layer)
        mid = lo + int((hi - lo) * 0.62)
        plan.spread(stats, lo, mid)
        plan.spread(ops, mid, hi)

    def send(b, job):
        plan.spread([part(start, *outputs(b))], job[0] + 8, job[0] + 9)

    plan.now(part(start, ("coefs", 0), ("h0", 0), ("kv0", 0), ("kv0", 1), ("h0", 1), ("kv0", 2),
                  ("kv0", 3), ("q", 0), ("h", 1), *[("w", c) for c in range(NUM_CHUNKS)], ("wd", 0), ("kv", 1),
                  ("h", 2), ("h", 3), ("kv", 2), ("q", 1)),
             forward_table, part(wait, ("coefs", 0)), broadcast_coefs, inverse_table)
    plan.cut(part(wait, ("h0", 0)))
    add_transform(filter_spectra, 0, [0])
    plan.now(part(wait, ("kv0", 0), ("kv0", 1)), *kv_pieces(0, [0]))
    add_transform(signal_spectra, 0, [0])
    plan.cut(part(wait, ("h0", 1)))
    plan.spread(conv_pieces(0, [0]), *add_transform(filter_spectra, 0, [1]))
    plan.now(part(wait, ("kv0", 2), ("kv0", 3)), *kv_pieces(0, [1]))
    add_transform(signal_spectra, 0, [1])
    plan.cut()
    plan.spread(conv_pieces(0, [1]), *add_transform(inverse, 0, [0]))
    plan.now(part(wait, ("q", 0)))
    stats, ops = norm_pieces(0, 0)
    plan.spread(stats[:len(stats) // 2], *add_transform(inverse, 0, [1]))
    plan.cut(part(wait, ("h", 1)))
    plan.spread(stats[len(stats) // 2:], *add_transform(filter_spectra, 1))
    plan.now(part(wait, ("w", 0)), plan.unpin, *ops[:16])
    for n, piece in enumerate(transpose_pieces(0, pin=True)):
        plan.now(piece, *ops[16 + 6 * n:22 + 6 * n])
    plan.now(plan.unpin, *gate_up_weight_pieces(0))

    for chunks, arrivals, prepare in (((0,), (1,), (1,)), ((1,), (2, 3), (2,)), ((2,), (4, 5), (3, 4)),
                                      ((3, 4), (6,), (5, 6))):
        plan.cut(part(wait, *[("w", n) for n in arrivals]))
        lo, hi = add_gate_up(chunks, busy=0.4)
        if prepare[0] in arrivals:
            plan.spread(transpose_pieces(prepare[0]), lo, lo + 2)
            lo += 5
        plan.spread([piece for n in prepare for piece in gate_up_weight_pieces(n, pin=n in arrivals)], lo, hi - 1)
        plan.spread([piece for n in arrivals if n > prepare[0] for piece in transpose_pieces(n)], lo,
                    lo + 20 if len(prepare) > 1 else hi - 2)
    plan.cut(part(wait, ("wd", 0)))
    lo, hi = add_gate_up((5, 6))
    plan.spread([piece for r in DOWN_ORDER[:4] for piece in down_weight_pieces(r)], lo, hi - 1)
    plan.cut(part(wait, ("kv", 1), ("h", 2), ("h", 3)))
    lo, hi = add_down(0, 0)
    for n, r in enumerate(DOWN_ORDER[4:]):
        plan.spread(down_weight_pieces(r), lo + n * DOWN_PASSES, lo + (n + 1) * DOWN_PASSES)
    plan.spread(kv_pieces(1), lo + DOWN_PASSES, lo + 5 * DOWN_PASSES + 10)
    add_transform(filter_spectra, 2)
    add_transform(filter_spectra, 3)
    add_transform(signal_spectra, 1)
    stats, ops = norm_pieces(0, 1)
    plan.spread([piece for piece in stats if piece.args[-2] < 2], lo + 5 * DOWN_PASSES + 5, hi + 3)
    plan.spread([piece for piece in stats if piece.args[-2] >= 2], hi + 1, hi + 15)
    plan.spread(ops, hi + 15, plan.planned - 1)

    plan.cut(part(wait, ("kv", 2), ("q", 1)))
    lo, _ = add_gate_up()
    add_transform(signal_spectra, 2)
    plan.spread(kv_pieces(2), lo, lo + 2 * GATE_UP_PASSES)
    plan.spread(conv_pieces(1), lo + 2 * GATE_UP_PASSES, plan.planned)
    plan.cut()
    inv = add_transform(inverse, 1)
    _, hi = add_down(0, 1)
    spread_norm(1, 0, inv[1], hi - 12)
    conv = conv_pieces(2)
    split = len(conv) // 5 // 6 * 6
    plan.spread(conv[:split], inv[0], hi)

    plan.cut()
    job = add_gate_up()
    plan.spread(conv[split:], *job)
    send(0, job)
    plan.cut()
    inv = add_transform(inverse, 2)
    lo, hi = add_down(1, 0)
    add_transform(signal_spectra, 3)
    spread_norm(2, 0, inv[1], hi + 8)
    plan.spread(kv_pieces(3, [0]), inv[0], lo + 30)
    plan.spread(kv_pieces(3, [1]), lo + 30, hi)

    plan.cut()
    conv = conv_pieces(3)
    split = 2 * len(conv) // 5 // 6 * 6
    plan.spread(conv[:split], *add_gate_up())
    lo, hi = add_down(2, 0)
    spread_norm(1, 1, lo, hi - 12)
    plan.spread(conv[split:-split], lo, hi)
    plan.spread(conv[-split:], *add_gate_up())
    inv = add_transform(inverse, 3)
    _, hi = add_down(1, 1)
    spread_norm(3, 0, inv[1], hi - 12)

    plan.cut()
    send(1, add_gate_up())
    lo, hi = add_down(3, 0)
    spread_norm(2, 1, lo, hi - 12)
    add_gate_up()
    lo, hi = add_down(2, 1)
    spread_norm(3, 1, lo, hi - 12)
    plan.cut()
    send(2, add_gate_up())
    add_down(3, 1)
    plan.now(part(wait, *[name for b in range(NUM_BLOCKS) for name in outputs(b)]))

    plan.run()
    assert not in_flight


def _run(A_q, A_k, A_v, A_shift_k, A_ssm_k, A_ssm_D, B_x, B_w_gate, B_w_up, B_w_down):
    del B_x
    batch, S, D = A_q.shape
    F = B_w_gate.shape[1]
    taps = A_shift_k.shape[1]
    assert (batch, S, D, F) == (1, NUM_BLOCKS * BLOCK, 7 * HALF, NUM_CHUNKS * CHUNK)
    tiles, rest = S // LANES, NUM_CHUNKS - 2 * PAIRS
    hbm = pl.BlockSpec(memory_space=pltpu.HBM)
    folded = lambda *lead: pltpu.VMEM(lead + (SUB, 2 * LANES), BF16)
    out = pl.pallas_call(
        _kernel,
        out_shape=jax.ShapeDtypeStruct((D, S), BF16),
        in_specs=[hbm] * 9,
        out_specs=hbm,
        scratch_shapes=[
            *[pltpu.VMEM(shape, BF16) for shape in ((taps, D), (D,), (LANES, 2 * LANES), (2 * LANES, LANES))],
            *[pltpu.VMEM((D, S), BF16)] * 4,
            *[pltpu.VMEM((D, F), BF16)] * 3,
            pltpu.VMEM((D, S), BF16),
            pltpu.VMEM((taps + 1, D, LANES), F32),
            pltpu.VMEM((tiles, 6, D, LANES), F32),
            pltpu.VMEM((NUM_BLOCKS - 1, 2, D, LANES), F32),
            folded(tiles, D // PACKED),
            pltpu.VMEM((tiles, D, 2 * LANES), BF16),
            [pltpu.VMEM((4, D, LANES), F32)] * NUM_BLOCKS,
            [pltpu.VMEM((2, 2, len(WEIGHT_TILES), HALF, LANES), U32)] * NUM_CHUNKS,
            [[folded(3 if r in SHORT else 7, SUB) for r in range(7)]] * NUM_CHUNKS,
            [folded(7, PAIRS + 1, D // 4 // PACKED)] * 7,
            [folded(rest, 2, D // 4 // PACKED)] * 7,
            [pltpu.VMEM((D, BLOCK), F32)] * NUM_BLOCKS,
            folded(RHS_START[7], SUB),
            [folded(7, 7, SUB)] * PAIRS,
            [folded(7, 2, SUB)] * rest,
            pltpu.SMEM((1,), jnp.int32),
            pltpu.SemaphoreType.DMA((56,)),
        ],
        compiler_params=pltpu.CompilerParams(
            vmem_limit_bytes=120 * 2**20, disable_bounds_checks=True, disable_semaphore_checks=True),
    )(A_q[0].T, A_k[0].T, A_v[0].T, A_shift_k.T, A_ssm_k, A_ssm_D, B_w_gate, B_w_up, B_w_down.T)
    return out.T[None]


@jax.jit
def pallas_interleave_layers__ssm_conv_h3__geglu_ffn__prompt_kernel(
    A_q: jax.Array,
    A_k: jax.Array,
    A_v: jax.Array,
    A_shift_k: jax.Array,
    A_ssm_k: jax.Array,
    A_ssm_D: jax.Array,
    B_x: jax.Array,
    B_w_gate: jax.Array,
    B_w_up: jax.Array,
    B_w_down: jax.Array,
):
    return _run(A_q, A_k, A_v, A_shift_k, A_ssm_k, A_ssm_D, B_x, B_w_gate, B_w_up, B_w_down)
```

```python
import functools

import jax
import jax.experimental.pallas as pl
import jax.experimental.pallas.tpu as pltpu
import jax.numpy as jnp
import numpy as np

F32, BF16, U32 = jnp.float32, jnp.bfloat16, jnp.uint32
LANES, HALF, SUB, PACKED = 128, 64, 8, 16
BLOCK = 4 * LANES
CHUNK = 2 * LANES
NUM_BLOCKS, NUM_CHUNKS = 4, 7
PAIRS = 2
EPS = 1e-5

GELU_SCALE = float((np.sqrt(2.0 / np.pi) * 0.044715) ** (1.0 / 3.0))
GELU_LINEAR = float(np.sqrt(2.0 / np.pi) / GELU_SCALE)
DOWN_SCALE = 0.5 / GELU_SCALE ** 2

LHS_TERMS = ((0, 1, 3), (2, 1, 3), (0, 0, 0), (3, 0, 0), (0, 1, 1), (2, -1, 0), (1, -1, 3))
RHS_TERMS = ((0, 1, 3), (0, 0, 0), (1, -1, 3), (2, -1, 0), (3, 0, 0), (0, 1, 1), (2, 1, 3))
OUT_TERMS = ({0: 1, 3: 1, 4: -1, 6: 1}, {2: 1, 4: 1}, {1: 1, 3: 1}, {0: 1, 1: -1, 2: 1, 5: 1})
GATE_UP_ORDER = (2, 4, 1, 3, 0, 6, 5)
DOWN_ORDER = (2, 4, 0, 1, 5, 3, 6)

SHORT = (3, 4, 6)
RHS_START = tuple(sum(4 if x in SHORT else 7 for x in range(r)) for r in range(8))
WEIGHT_TILES = ((0, 1), (2, 3), (4, 5), (6, 6), (2, 2))

GATE_UP_PASSES = sum(6 if r in SHORT else 7 for r in range(7))
DOWN_PASSES = 7 * PAIRS + 4 * (NUM_CHUNKS - 2 * PAIRS)


def _tile(j):
    return slice(j * LANES, (j + 1) * LANES)


def _combine(term, quadrant):
    a, sign, b = term
    a = quadrant(a)
    b = quadrant(b) if sign else None
    if b is None:
        return a
    if a is None:
        assert sign > 0
        return b
    return a + b if sign > 0 else a - b


def _inner_sum(product):
    m1, m2, m3, m4, m5, m6, m7 = (product(s) for s in range(7))
    return [(m1 + m4) - m5 + m7, m3 + m5, m2 + m4, (m1 - m2) + m3 + m6]


def _outer_sum(product, order, emit):
    m = {}
    for r in order:
        m[r] = product(r)
        for quadrant, terms in enumerate(OUT_TERMS):
            if r in terms and all(x in m for x in terms):
                names = sorted(terms, key=lambda x: (x != r, terms[x] < 0))
                if terms[names[0]] < 0:
                    names[0], names[1] = names[1], names[0]
                blocks = list(m[names[0]])
                for x in names[1:]:
                    blocks = [u + v if terms[x] > 0 else u - v for u, v in zip(blocks, m[x])]
                emit(quadrant, blocks)


def _fold(x):
    x = x.reshape(x.shape[0] // PACKED, 2, SUB, LANES)
    return jnp.concatenate([x[:, 0], x[:, 1]], axis=-1).astype(BF16)


def _unfold(v):
    return jnp.stack([v[:, :, :LANES], v[:, :, LANES:]], axis=1).reshape(PACKED * v.shape[0], LANES)


def _low_lanes(shape):
    return jax.lax.broadcasted_iota(jnp.int32, shape, 1) < HALF


def _zip_halves(a, b):
    a, b = pltpu.bitcast(a, U32), pltpu.bitcast(b, U32)
    low = _low_lanes(a.shape)
    swap = pltpu.roll(jnp.where(low, b, a), HALF, 1)
    return [pltpu.bitcast(v, BF16).astype(F32) for v in (jnp.where(low, a, swap), jnp.where(low, swap, b))]


def _geglu(gate_up):
    g, u = gate_up[:HALF], gate_up[HALF:]
    return (g * u) * (1.0 + jnp.tanh(g * (GELU_LINEAR + g * g)))


class _Schedule:
    def __init__(self, table_ref, mark_ref):
        self.table_ref, self.mark_ref = table_ref, mark_ref
        self.steps, self.room, self.pending = [], [], {}
        self.slot = 0
        self.reset()

    def reset(self):
        self.token = self.last = self._never = self._zero = None

    def unpin(self):
        self.token = self.last = None

    @property
    def planned(self):
        return len(self.room)

    def add(self, room, fn, *args):
        self.room.extend(room)
        self.steps.append(functools.partial(fn, *args))

    def now(self, *pieces):
        self.steps.extend(pieces)

    def cut(self, *transfers):
        if transfers:
            self.now(self._block_end, *transfers)
        self.now(self._block_end)

    def _block_end(self):
        def tick(i, carry):
            self.mark_ref[0] = i
            return carry

        jax.lax.fori_loop(0, 2, tick, 0)
        self.reset()

    def spread(self, pieces, lo, hi):
        weight = np.cumsum(self.room[lo:hi])
        for n, piece in enumerate(pieces):
            at = int(np.searchsorted(weight, (n + 0.5) / len(pieces) * weight[-1]))
            self.pending.setdefault(lo + at, []).append(piece)

    def never(self):
        if self._never is None:
            self._never = self.table_ref[0:PACKED, :LANES].astype(F32)[:SUB] > 2.0
        return self._never

    def after(self, x):
        if self.token is None:
            return x
        token = self.token if self.token.dtype == x.dtype else pltpu.bitcast(self.token, x.dtype)
        return jnp.where(self.never()[:x.shape[0]], token[:x.shape[0]], x)

    def zero(self):
        if self._zero is None:
            self._zero = jnp.where(self.never(), SUB, 0)[0, 0]
        return self._zero

    def dot(self, lhs, rhs):
        pieces = self.pending.pop(self.slot, ())
        for n, piece in enumerate(pieces):
            if self.last is not None:
                regs = self.last.shape[0] // SUB
                if regs <= PACKED:
                    row = (self.slot % 4 * len(pieces) + n) * regs // (4 * len(pieces)) * SUB
                else:
                    row = n * regs // len(pieces) * SUB
                self.token = self.last[row:row + SUB, :LANES]
            piece()
        self.slot += 1
        self.last = jnp.dot(lhs(), rhs(), preferred_element_type=F32)
        return self.last

    def run(self):
        for step in self.steps:
            step()
        assert not self.pending


def _kernel(q_hbm, k_hbm, v_hbm, taps_hbm, h_hbm, skip_hbm, wg_hbm, wu_hbm, wd_hbm,
            o_hbm,
            taps_v, skip_v, fwd_v, inv_v, q_v, k_v, v_v, h_v, wg_v, wu_v, wd_v, o_v,
            coef, spectra, h_prev, kv_s, y_freq, y_s, w_t, w_gu, wd_pair, wd_rest, x_s,
            h_ops, act_pair, act_rest, mark, sems):
    D = q_v.shape[0]
    DH, DQ = D // 2, D // 4
    taps = taps_v.shape[0]
    part = functools.partial
    plan = _Schedule(fwd_v, mark)
    dot, after = plan.dot, plan.after

    sem_ids, in_flight = {}, []

    def copies(name):
        kind, n = name[:2]
        every = slice(None)
        kv_pair = ((k_hbm, k_v), (v_hbm, v_v))
        if kind == "coefs":
            views = [(p, ...) for p in ((taps_hbm, taps_v), (skip_hbm, skip_v))]
        elif kind == "kv0":
            views = [(p, (slice(n * DQ, (n + 1) * DQ), slice(0, BLOCK))) for p in kv_pair]
        elif kind == "h0":
            views = [((h_hbm, h_v), (slice(n * DH, (n + 1) * DH), slice(0, BLOCK)))]
        elif kind == "kv":
            cols = slice(BLOCK, 2 * BLOCK) if n == 1 else slice(2 * BLOCK, None)
            views = [(p, (every, cols)) for p in kv_pair]
        elif kind == "h":
            views = [((h_hbm, h_v), (every, slice(n * BLOCK, (n + 1) * BLOCK)))]
        elif kind == "q":
            views = [((q_hbm, q_v), (every, slice(0, BLOCK) if n == 0 else slice(BLOCK, None)))]
        elif kind == "w":
            views = [(p, (every, slice(n * CHUNK, (n + 1) * CHUNK))) for p in ((wg_hbm, wg_v), (wu_hbm, wu_v))]
        elif kind == "wd":
            views = [((wd_hbm, wd_v), (every, every))]
        else:
            i, k = divmod(name[2], 2)
            col = n * BLOCK + k * CHUNK
            views = [((o_v, o_hbm), (slice(i * DH, (i + 1) * DH), slice(col, col + CHUNK)))]
        return [pltpu.make_async_copy(src.at[idx], dst.at[idx], sems.at[sem_ids.setdefault((name, i), len(sem_ids))])
                for i, ((src, dst), idx) in enumerate(views)]

    def start(*names):
        for name in names:
            in_flight.append(name)
            for copy in copies(name):
                copy.start()

    def wait(*names):
        for name in names:
            in_flight.remove(name)
            for copy in copies(name):
                copy.wait()

    def outputs(b):
        return [("out", b, m) for m in range(4)]

    def broadcast_coefs():
        rows = taps_v[...].astype(F32)
        for j in range(taps):
            coef[j] = jnp.broadcast_to(rows[j:j + 1], (LANES, D)).T
        coef[taps] = jnp.broadcast_to(skip_v[...].astype(F32).reshape(1, D), (LANES, D)).T

    def forward_table():
        n = jax.lax.broadcasted_iota(jnp.int32, (LANES, LANES), 0)
        k = jax.lax.broadcasted_iota(jnp.int32, (LANES, LANES), 1)
        angle = (((4 * k + 1) * n) & (4 * LANES - 1)).astype(F32) * (np.pi / (2 * LANES))
        fwd_v[:, :LANES] = jnp.cos(angle).astype(BF16)
        fwd_v[:, LANES:] = jnp.sin(angle).astype(BF16)

    def inverse_table():
        inv_v[...] = (fwd_v[...].astype(F32).T * (1.0 / LANES)).astype(BF16)

    def transpose_pieces(c, pin=False):
        def piece(m, i):
            w = (wg_v, wu_v)[m]
            groups = [w[u * HALF:(u + 1) * HALF, _tile(2 * c + i)] for pair in WEIGHT_TILES for u in pair]
            words = pltpu.bitcast(jnp.concatenate(groups, axis=0).T, U32)
            for j in range(len(WEIGHT_TILES)):
                w_t[c][m, i, j] = words[:, _tile(j)]
            if pin:
                plan.token = words[:SUB, :LANES]

        return [part(piece, m, i) for m in range(2) for i in range(2)]

    def gate_up_weight_pieces(c, pin=False):
        def piece(m, g, products):
            @functools.cache
            def raw(i, e, j):
                at = e * HALF // 2 + g * SUB
                if pin:
                    words = after(w_t[c][m, i, j, pl.ds(pl.multiple_of(at + plan.zero(), SUB), SUB)])
                else:
                    words = w_t[c][m, i, j, at:at + SUB]
                return pltpu.bitcast(words, BF16).astype(F32)

            for r in products:
                low = _low_lanes((PACKED, LANES))
                at = m * HALF // PACKED + g

                def put(s, val):
                    w_gu[c][r][s, at:at + 1] = _fold(val)

                def padded(e, a, n):
                    j = 2 * (n % 2) + a
                    return jnp.where(low, raw(n // 2, e, j), 0.0) if j == 3 else raw(n // 2, e, j)

                if r in SHORT:
                    head = [_combine(LHS_TERMS[r], lambda n: raw(n // 2, e, (0, 2)[n % 2])) for e in range(2)]
                    tail = [_combine(LHS_TERMS[r], lambda n: raw(n // 2, e, (4, 3)[n % 2])) for e in range(2)]
                    put(0, head[0] - jnp.where(low, 0.0, head[1]))
                    put(1, jnp.where(low, head[1], tail[1] - tail[0]))
                    put(2, jnp.where(low, tail[0], head[1]))
                else:
                    quads = [_combine(LHS_TERMS[r], part(padded, e, a)) for e in range(2) for a in range(2)]
                    for s in range(7):
                        put(s, _combine(LHS_TERMS[s], quads.__getitem__))

        groups = range(HALF // PACKED)
        if pin:
            return [part(piece, m, g, rs) for m in range(2) for rs in ((2, 4), (1, 3), (0, 6), (5,)) for g in groups]
        return [part(piece, m, g, (r,)) for m in range(2) for g in groups for r in (0, 1, 3, 6, 5, 2, 4)]

    def down_weight_pieces(r):
        def rows(i, e, g):
            r0 = i * DH + e * DQ + PACKED * g
            return slice(r0, r0 + PACKED)

        def paired(j, g):
            scale = after(jnp.full((1, LANES), DOWN_SCALE, F32))

            def pick(e, n):
                i, f = divmod(n, 2)
                at = rows(i, e, g)
                return jnp.stack(_zip_halves(wd_v[at, _tile(4 * j + f)], wd_v[at, _tile(4 * j + 2 + f)]))

            left = [scale * _combine(LHS_TERMS[r], part(pick, e)) for e in range(2)]
            for s in range(7):
                wd_pair[r][s, j, g:g + 1] = _fold(_combine(LHS_TERMS[s], lambda n: left[n // 2][n % 2]))

        def single(c, e):
            scale = after(jnp.full((1, LANES), DOWN_SCALE, F32))
            for g in range(DQ // PACKED):
                pick = lambda n: wd_v[rows(n // 2, e, g), _tile(2 * c + n % 2)].astype(F32)
                wd_rest[r][c - 2 * PAIRS, e, g:g + 1] = _fold(scale * _combine(LHS_TERMS[r], pick))

        return ([part(paired, j, g) for j in range(PAIRS) for g in range(DQ // PACKED)]
                + [part(single, c, e) for e in range(2) for c in range(2 * PAIRS, NUM_CHUNKS)])

    def kv_pieces(b, halves=(0, 1)):
        def piece(j, r0):
            rows = slice(r0, r0 + PACKED)
            lane = after(jax.lax.broadcasted_iota(jnp.int32, (SUB, LANES), 1))
            cur = pltpu.bitcast(k_v[rows, _tile(j)], U32)
            prev = pltpu.bitcast(k_v[rows, _tile(j - 1)], U32) if j else jnp.zeros_like(cur)
            shifted = pltpu.bitcast(cur, BF16).astype(F32) * coef[0, rows, :]
            for t in range(1, taps):
                moved = pltpu.roll(jnp.where(lane >= LANES - t, prev, cur), t, 1)
                shifted = shifted + pltpu.bitcast(moved, BF16).astype(F32) * coef[t, rows, :]
            kv_s[j, r0 // PACKED:r0 // PACKED + 1] = _fold(shifted * v_v[rows, _tile(j)].astype(F32))

        return [part(piece, 4 * b + n, i * DH + r0) for i in halves for n in range(4) for r0 in range(0, DH, PACKED)]

    def filter_spectra(b, i):
        rows = slice(i * DH, (i + 1) * DH)
        prev = (h_prev[b - 1, 0, rows, :], h_prev[b - 1, 1, rows, :]) if b else None
        for j in range(4 * b, 4 * b + 4):
            freq = dot(lambda: h_v[rows, _tile(j)], lambda: fwd_v[...])
            re, im = freq[:, :LANES], freq[:, LANES:]
            if j == 0:
                re = re + coef[taps, rows, :]
            c, d = (re + prev[1], im - prev[0]) if prev else (re, im)
            prev = (re, im)
            spectra[j, 0, rows, :], spectra[j, 1, rows, :], spectra[j, 2, rows, :] = c, d - c, c + d
        if b + 1 < NUM_BLOCKS:
            h_prev[b, 0, rows, :], h_prev[b, 1, rows, :] = prev

    def signal_spectra(b, i):
        rows = slice(i * DH, (i + 1) * DH)
        for j in range(4 * b, 4 * b + 4):
            freq = dot(lambda: _unfold(kv_s[j, i * DH // PACKED:(i + 1) * DH // PACKED]), lambda: fwd_v[...])
            re, im = freq[:, :LANES], freq[:, LANES:]
            spectra[j, 3, rows, :], spectra[j, 4, rows, :], spectra[j, 5, rows, :] = re + im, re, im

    def conv_pieces(b, halves=(0, 1)):
        state = {}

        def plane(hi, r0, p, js):
            rows = slice(r0, r0 + SUB)
            for j in js:
                newer = state["h"] if j else spectra[hi, p, rows, :]
                signal = spectra[j, 3 + p, rows, :]
                terms = {1: newer * signal}
                if j < hi:
                    state["h"] = spectra[hi - 1 - j, p, rows, :]
                    terms[0] = state["h"] * signal
                for n, term in terms.items():
                    if j == 0 and p == 0:
                        state[n] = after(term)
                        continue
                    base = state["shared", n] if j == 0 else state[n]
                    base = after(base) if j == js[0] else base
                    state[n] = base - term if p == 2 else base + term
            if js[-1] == hi:
                for n in range(2):
                    if p == 0:
                        state["shared", n] = state[n]
                    else:
                        y_freq[hi - 1 + n, rows, _tile(2 - p)] = state[n].astype(BF16)

        runs = lambda hi: [range(hi + 1)] if hi < 8 else [range((hi + 1) // 2), range((hi + 1) // 2, hi + 1)]
        return [part(plane, hi, r0, p, js) for i in halves for hi in (4 * b + 1, 4 * b + 3)
                for r0 in range(i * DH, (i + 1) * DH, SUB) for p in range(3) for js in runs(hi)]

    def inverse(b, i):
        rows = slice(i * DH, (i + 1) * DH)
        for j in range(4 * b, 4 * b + 4):
            y_s[b][j % 4, rows, :] = dot(lambda: y_freq[j, rows, :], lambda: inv_v[...])

    def norm_pieces(b, layer):
        state = {}

        def fetch(stage, t, r0, size):
            if layer == 0 and stage < 3:
                return q_v[r0:r0 + size, _tile(4 * b + t)].astype(F32)
            if (b, layer) == (0, 0):
                return x_s[b][r0:r0 + size, _tile(t)]
            return x_s[b][pl.ds(pl.multiple_of(r0 + stage * plan.zero(), SUB), size), _tile(t)]

        def average(t, r0, val):
            for i in range(0, HALF, SUB):
                state["sum", t] = state["sum", t] + val[i:i + SUB] if r0 + i else val[:SUB]
            return jnp.sum(state["sum", t], axis=0, keepdims=True) * (1.0 / D) if r0 + HALF == D else None

        def center(t, r0):
            x = fetch(0, t, r0, HALF)
            state["mean", t] = average(t, r0, jnp.concatenate([after(x[:SUB]), x[SUB:]], axis=0))

        def deviation(stage, t, r0):
            centered = fetch(stage, t, r0, HALF) - after(state["mean", t])
            var = average(t, r0, centered * centered)
            if var is not None:
                state["scale", t] = jax.lax.rsqrt(var + EPS) * (GELU_SCALE if stage == 3 else 1.0)

        def gate(t, r0):
            rows = slice(r0, r0 + HALF)
            x = fetch(2, t, r0, HALF)
            x = x + (x - after(state["mean", t])) * state["scale", t] * y_s[b][t, rows, :]
            x_s[b][rows, _tile(t)] = x
            mean = average(t, r0, x)
            if mean is not None:
                state["mean", t] = mean

        def operands(u, r0, products):
            mean = functools.cache(lambda t: after(state["mean", t]))
            at = (u * HALF + r0) // PACKED

            @functools.cache
            def normed(j, a, t):
                row = (4 * j + 2 * a + u) * HALF + r0
                return (fetch(4 + products[0], t, row, PACKED) - mean(t)) * state["scale", t] if row < D else None

            for r in products:
                right = lambda a, t: _combine(RHS_TERMS[r], lambda n: normed(n // 2, a, 2 * (n % 2) + t))
                if r in SHORT:
                    for t in range(2):
                        for a in range(2 - u):
                            h_ops[RHS_START[r] + 2 * t + a, at:at + 1] = _fold(right(a, t))
                else:
                    quads = [right(a, t) for a in range(2) for t in range(2)]
                    for s in range(7):
                        h_ops[RHS_START[r] + s, at:at + 1] = _fold(_combine(RHS_TERMS[s], quads.__getitem__))

        stages = (center, part(deviation, 1), gate, part(deviation, 3))
        return ([part(stage, t, r0) for stage in stages for t in range(4) for r0 in range(0, D, HALF)],
                [part(operands, u, r0, rs) for rs in ((0,), (1, 3), (5,), (2,), (4, 6))
                 for u in range(2) for r0 in range(0, HALF, PACKED)])

    def gate_up(c, defer):
        def product(r):
            lhs = lambda s: lambda: _unfold(w_gu[c][r][s])
            at = RHS_START[r]
            if r not in SHORT:
                return _inner_sum(lambda s: dot(lhs(s), lambda: _unfold(h_ops[at + s])))
            out = [None] * 4
            for t in range(2):
                first, second = at + 2 * t, at + 2 * t + 1
                join = lambda a, b: _unfold(jnp.concatenate([a, b], axis=0))
                shared = dot(lhs(2), lambda: join(h_ops[second, 0:4], h_ops[first, 4:8]))
                out[t] = dot(lhs(0), lambda: _unfold(h_ops[first])) + shared
                out[2 + t] = dot(lhs(1), lambda: join(h_ops[first, 0:4], h_ops[second, 0:4])) + shared
            return out

        acts = {}
        _outer_sum(product, GATE_UP_ORDER, lambda m, blocks: acts.update({m: [_geglu(v) for v in blocks]}))

        def operands(r, g0, g1, late):
            def quadrant(n, m):
                x = acts[m ^ 1][n][PACKED * g0:PACKED * g1]
                if late and m == RHS_TERMS[r][0]:
                    x = jnp.concatenate([after(x[i:i + SUB]) for i in range(0, x.shape[0], SUB)], axis=0)
                return x

            right = [_combine(RHS_TERMS[r], part(quadrant, n)) for n in range(4)]
            if c < 2 * PAIRS:
                at = 4 * (c % 2)
                for s in range(7):
                    act_pair[c // 2][r, s, at + g0:at + g1] = _fold(_combine(RHS_TERMS[s], right.__getitem__))
            else:
                for n in range(4):
                    at = 4 * (n // 2)
                    act_rest[c - 2 * PAIRS][r, n % 2, at + g0:at + g1] = _fold(right[n])

        for r in range(7):
            if r not in defer:
                operands(r, 0, 4, False)
        if defer:
            plan.spread([part(operands, r, g, g + 1, True) for r in defer for g in range(4)],
                        plan.slot + 3, plan.slot + 11)

    def down(b, layer):
        def product(r):
            one = lambda s, j: dot(lambda: _unfold(wd_pair[r][s, j]), lambda: _unfold(act_pair[j][r, s]))
            out = _inner_sum(lambda s: functools.reduce(jnp.add, [one(s, j) for j in range(PAIRS)]))
            rest = lambda n, c: dot(lambda: _unfold(wd_rest[r][c, n // 2]), lambda: _unfold(act_rest[c][r, n % 2]))
            return [functools.reduce(jnp.add, [out[n]] + [rest(n, c) for c in range(len(act_rest))]) for n in range(4)]

        end = plan.slot + 7 * DOWN_PASSES

        def emit(m, blocks):
            for n, val in enumerate(blocks):
                r0 = (m // 2) * DH + (n // 2) * DQ
                rows, t = slice(r0, r0 + DQ), 2 * (1 - m % 2) + n % 2
                val = x_s[b][rows, _tile(t)] + val
                if layer == 0:
                    x_s[b][rows, _tile(t)] = val
                else:
                    o_v[rows, _tile(4 * b + t)] = val.astype(BF16)
            if layer == 1 and b == NUM_BLOCKS - 1:
                if plan.slot < end:
                    plan.pending.setdefault(plan.slot + 8, []).append(part(start, ("out", b, m ^ 1)))
                else:
                    start(("out", b, m ^ 1))

        _outer_sum(product, DOWN_ORDER, emit)

    def add_gate_up(chunks=range(NUM_CHUNKS), busy=0.1):
        lo = plan.planned
        room = [busy if 9 <= i < 15 or 22 <= i < 28 or i >= 35 else 1.0 for i in range(GATE_UP_PASSES)]
        for c in chunks:
            plan.add(room, gate_up, c, () if c + 1 == NUM_CHUNKS else (3, 6))
        return lo, plan.planned

    def add_down(b, layer):
        lo = plan.planned
        plan.add([1.0] * (7 * DOWN_PASSES), down, b, layer)
        return lo, plan.planned

    def add_transform(fn, b, halves=(0, 1)):
        lo = plan.planned
        for i in halves:
            plan.add([4.0] * 4, fn, b, i)
        return lo, plan.planned

    def spread_norm(b, layer, lo, hi):
        stats, ops = norm_pieces(b, layer)
        mid = lo + int((hi - lo) * 0.62)
        plan.spread(stats, lo, mid)
        plan.spread(ops, mid, hi)

    def send(b, job):
        plan.spread([part(start, *outputs(b))], job[0] + 8, job[0] + 9)

    plan.now(part(start, ("coefs", 0), ("h0", 0), ("kv0", 0), ("kv0", 1), ("h0", 1), ("kv0", 2),
                  ("kv0", 3), ("q", 0), ("h", 1), *[("w", c) for c in range(NUM_CHUNKS)], ("wd", 0), ("kv", 1),
                  ("h", 2), ("h", 3), ("kv", 2), ("q", 1)),
             forward_table, part(wait, ("coefs", 0)), broadcast_coefs, inverse_table)
    plan.cut(part(wait, ("h0", 0)))
    add_transform(filter_spectra, 0, [0])
    plan.now(part(wait, ("kv0", 0), ("kv0", 1)), *kv_pieces(0, [0]))
    add_transform(signal_spectra, 0, [0])
    plan.cut(part(wait, ("h0", 1)))
    plan.spread(conv_pieces(0, [0]), *add_transform(filter_spectra, 0, [1]))
    plan.now(part(wait, ("kv0", 2), ("kv0", 3)), *kv_pieces(0, [1]))
    add_transform(signal_spectra, 0, [1])
    plan.cut()
    plan.spread(conv_pieces(0, [1]), *add_transform(inverse, 0, [0]))
    plan.now(part(wait, ("q", 0)))
    stats, ops = norm_pieces(0, 0)
    plan.spread(stats[:56], *add_transform(inverse, 0, [1]))
    plan.now(plan.unpin, *stats[56:77])
    plan.cut(part(wait, ("h", 1)))
    plan.spread(stats[77:] + ops[:8], *add_transform(filter_spectra, 1))
    plan.now(part(wait, ("w", 0)), plan.unpin, *ops[8:16])
    for n, piece in enumerate(transpose_pieces(0, pin=True)):
        plan.now(piece, *ops[16 + 6 * n:22 + 6 * n])
    plan.now(plan.unpin, *gate_up_weight_pieces(0))

    for chunks, arrivals, prepare in (((0,), (1,), (1,)), ((1,), (2, 3), (2,)), ((2,), (4, 5), (3, 4)),
                                      ((3, 4), (6,), (5, 6))):
        plan.cut(part(wait, *[("w", n) for n in arrivals]))
        lo, hi = add_gate_up(chunks, busy=0.4)
        if prepare[0] in arrivals:
            plan.spread(transpose_pieces(prepare[0]), lo, lo + 2)
            lo += 5
        plan.spread([piece for n in prepare for piece in gate_up_weight_pieces(n, pin=n in arrivals)], lo, hi - 1)
        plan.spread([piece for n in arrivals if n > prepare[0] for piece in transpose_pieces(n)], lo,
                    lo + 20 if len(prepare) > 1 else hi - 2)
    plan.cut(part(wait, ("wd", 0)))
    lo, hi = add_gate_up((5, 6))
    plan.spread([piece for r in DOWN_ORDER[:4] for piece in down_weight_pieces(r)], lo, hi - 1)
    plan.cut(part(wait, ("kv", 1), ("h", 2), ("h", 3)))
    lo, hi = add_down(0, 0)
    for n, r in enumerate(DOWN_ORDER[4:]):
        plan.spread(down_weight_pieces(r), lo + n * DOWN_PASSES, lo + (n + 1) * DOWN_PASSES)
    plan.spread(kv_pieces(1), lo + DOWN_PASSES, lo + 5 * DOWN_PASSES + 10)
    add_transform(filter_spectra, 2)
    add_transform(filter_spectra, 3)
    add_transform(signal_spectra, 1)
    stats, ops = norm_pieces(0, 1)
    plan.spread([piece for piece in stats if piece.args[-2] < 2], lo + 5 * DOWN_PASSES + 5, hi + 3)
    plan.spread([piece for piece in stats if piece.args[-2] >= 2], hi + 1, hi + 15)
    plan.spread(ops, hi + 15, plan.planned - 1)

    plan.cut(part(wait, ("kv", 2), ("q", 1)))
    lo, _ = add_gate_up()
    add_transform(signal_spectra, 2)
    plan.spread(kv_pieces(2), lo, lo + 2 * GATE_UP_PASSES)
    plan.spread(conv_pieces(1), lo + 2 * GATE_UP_PASSES, plan.planned)
    plan.cut()
    inv = add_transform(inverse, 1)
    _, hi = add_down(0, 1)
    spread_norm(1, 0, inv[1], hi - 12)
    conv = conv_pieces(2)
    split = len(conv) // 5 // 6 * 6
    plan.spread(conv[:split], inv[0], hi)

    plan.cut()
    job = add_gate_up()
    plan.spread(conv[split:], *job)
    send(0, job)
    inv = add_transform(inverse, 2)
    lo, hi = add_down(1, 0)
    add_transform(signal_spectra, 3)
    spread_norm(2, 0, inv[1], hi + 8)
    plan.spread(kv_pieces(3, [0]), inv[0], lo + 30)
    plan.spread(kv_pieces(3, [1]), lo + 30, hi)

    plan.cut()
    conv = conv_pieces(3)
    split = 2 * len(conv) // 5 // 6 * 6
    plan.spread(conv[:split], *add_gate_up())
    lo, hi = add_down(2, 0)
    spread_norm(1, 1, lo, hi - 12)
    plan.spread(conv[split:-split], lo, hi)
    plan.spread(conv[-split:], *add_gate_up())
    inv = add_transform(inverse, 3)
    _, hi = add_down(1, 1)
    spread_norm(3, 0, inv[1], hi - 12)

    plan.cut()
    send(1, add_gate_up())
    lo, hi = add_down(3, 0)
    spread_norm(2, 1, lo, hi - 12)
    add_gate_up()
    lo, hi = add_down(2, 1)
    spread_norm(3, 1, lo, hi - 12)
    send(2, add_gate_up())
    add_down(3, 1)
    plan.now(part(wait, *[name for b in range(NUM_BLOCKS) for name in outputs(b)]))

    plan.run()
    assert not in_flight


def _run(A_q, A_k, A_v, A_shift_k, A_ssm_k, A_ssm_D, B_x, B_w_gate, B_w_up, B_w_down):
    del B_x
    batch, S, D = A_q.shape
    F = B_w_gate.shape[1]
    taps = A_shift_k.shape[1]
    assert (batch, S, D, F) == (1, NUM_BLOCKS * BLOCK, 7 * HALF, NUM_CHUNKS * CHUNK)
    tiles, rest = S // LANES, NUM_CHUNKS - 2 * PAIRS
    hbm = pl.BlockSpec(memory_space=pltpu.HBM)
    folded = lambda *lead: pltpu.VMEM(lead + (SUB, 2 * LANES), BF16)
    out = pl.pallas_call(
        _kernel,
        out_shape=jax.ShapeDtypeStruct((D, S), BF16),
        in_specs=[hbm] * 9,
        out_specs=hbm,
        scratch_shapes=[
            *[pltpu.VMEM(shape, BF16) for shape in ((taps, D), (D,), (LANES, 2 * LANES), (2 * LANES, LANES))],
            *[pltpu.VMEM((D, S), BF16)] * 4,
            *[pltpu.VMEM((D, F), BF16)] * 3,
            pltpu.VMEM((D, S), BF16),
            pltpu.VMEM((taps + 1, D, LANES), F32),
            pltpu.VMEM((tiles, 6, D, LANES), F32),
            pltpu.VMEM((NUM_BLOCKS - 1, 2, D, LANES), F32),
            folded(tiles, D // PACKED),
            pltpu.VMEM((tiles, D, 2 * LANES), BF16),
            [pltpu.VMEM((4, D, LANES), F32)] * NUM_BLOCKS,
            [pltpu.VMEM((2, 2, len(WEIGHT_TILES), HALF, LANES), U32)] * NUM_CHUNKS,
            [[folded(3 if r in SHORT else 7, SUB) for r in range(7)]] * NUM_CHUNKS,
            [folded(7, PAIRS + 1, D // 4 // PACKED)] * 7,
            [folded(rest, 2, D // 4 // PACKED)] * 7,
            [pltpu.VMEM((D, BLOCK), F32)] * NUM_BLOCKS,
            folded(RHS_START[7], SUB),
            [folded(7, 7, SUB)] * PAIRS,
            [folded(7, 2, SUB)] * rest,
            pltpu.SMEM((1,), jnp.int32),
            pltpu.SemaphoreType.DMA((56,)),
        ],
        compiler_params=pltpu.CompilerParams(
            vmem_limit_bytes=120 * 2**20, disable_bounds_checks=True, disable_semaphore_checks=True),
    )(A_q[0].T, A_k[0].T, A_v[0].T, A_shift_k.T, A_ssm_k, A_ssm_D, B_w_gate, B_w_up, B_w_down.T)
    return out.T[None]


@jax.jit
def pallas_interleave_layers__ssm_conv_h3__geglu_ffn__prompt_kernel(
    A_q: jax.Array,
    A_k: jax.Array,
    A_v: jax.Array,
    A_shift_k: jax.Array,
    A_ssm_k: jax.Array,
    A_ssm_D: jax.Array,
    B_x: jax.Array,
    B_w_gate: jax.Array,
    B_w_up: jax.Array,
    B_w_down: jax.Array,
):
    return _run(A_q, A_k, A_v, A_shift_k, A_ssm_k, A_ssm_D, B_x, B_w_gate, B_w_up, B_w_down)
```

```python
import functools

import jax
import jax.experimental.pallas as pl
import jax.experimental.pallas.tpu as pltpu
import jax.numpy as jnp
import numpy as np

F32, BF16, U32 = jnp.float32, jnp.bfloat16, jnp.uint32
LANES, HALF, SUB, PACKED = 128, 64, 8, 16
BLOCK = 4 * LANES
CHUNK = 2 * LANES
NUM_BLOCKS, NUM_CHUNKS = 4, 7
LAST = 4 * NUM_BLOCKS - 1
PAIRS = 2
EPS = 1e-5

GELU_SCALE = float((np.sqrt(2.0 / np.pi) * 0.044715) ** (1.0 / 3.0))
GELU_LINEAR = float(np.sqrt(2.0 / np.pi) / GELU_SCALE)
DOWN_SCALE = 0.5 / GELU_SCALE ** 2

LHS_TERMS = ((0, 1, 3), (2, 1, 3), (0, 0, 0), (3, 0, 0), (0, 1, 1), (2, -1, 0), (1, -1, 3))
RHS_TERMS = ((0, 1, 3), (0, 0, 0), (1, -1, 3), (2, -1, 0), (3, 0, 0), (0, 1, 1), (2, 1, 3))
OUT_TERMS = ({0: 1, 3: 1, 4: -1, 6: 1}, {2: 1, 4: 1}, {1: 1, 3: 1}, {0: 1, 1: -1, 2: 1, 5: 1})
GATE_UP_ORDER = (2, 4, 1, 3, 0, 6, 5)
DOWN_ORDER = (2, 4, 0, 1, 5, 3, 6)

SHORT = (3, 4, 6)
RHS_START = tuple(sum(4 if x in SHORT else 7 for x in range(r)) for r in range(8))
WEIGHT_TILES = ((0, 1), (2, 3), (4, 5), (6, 6), (2, 2))

GATE_UP_PASSES = sum(6 if r in SHORT else 7 for r in range(7))
DOWN_PASSES = 7 * PAIRS + 4 * (NUM_CHUNKS - 2 * PAIRS)


def _tile(j):
    return slice(j * LANES, (j + 1) * LANES)


def _combine(term, quadrant):
    a, sign, b = term
    a = quadrant(a)
    b = quadrant(b) if sign else None
    if b is None:
        return a
    if a is None:
        assert sign > 0
        return b
    return a + b if sign > 0 else a - b


def _inner_sum(product):
    m1, m2, m3, m4, m5, m6, m7 = (product(s) for s in range(7))
    return [(m1 + m4) - m5 + m7, m3 + m5, m2 + m4, (m1 - m2) + m3 + m6]


def _outer_sum(product, order, emit):
    m = {}
    for r in order:
        m[r] = product(r)
        for quadrant, terms in enumerate(OUT_TERMS):
            if r in terms and all(x in m for x in terms):
                names = sorted(terms, key=lambda x: (x != r, terms[x] < 0))
                if terms[names[0]] < 0:
                    names[0], names[1] = names[1], names[0]
                blocks = list(m[names[0]])
                for x in names[1:]:
                    blocks = [u + v if terms[x] > 0 else u - v for u, v in zip(blocks, m[x])]
                emit(quadrant, blocks)


def _fold(x):
    x = x.reshape(x.shape[0] // PACKED, 2, SUB, LANES)
    return jnp.concatenate([x[:, 0], x[:, 1]], axis=-1).astype(BF16)


def _fold_all(parts):
    return _fold(jnp.concatenate(parts, axis=0)).reshape(len(parts), -1, SUB, 2 * LANES)


def _unfold(v):
    return jnp.stack([v[:, :, :LANES], v[:, :, LANES:]], axis=1).reshape(PACKED * v.shape[0], LANES)


def _load_tiles(ref, idx):
    @functools.cache
    def tiles():
        v = ref[idx]
        return v.shape[1] * PACKED, _unfold(v.reshape(-1, SUB, 2 * LANES))

    return functools.cache(lambda i: tiles()[1][i * tiles()[0]:(i + 1) * tiles()[0]])


def _low_lanes(shape):
    return jax.lax.broadcasted_iota(jnp.int32, shape, 1) < HALF


def _zip_halves(a, b):
    a, b = pltpu.bitcast(a, U32), pltpu.bitcast(b, U32)
    low = _low_lanes(a.shape)
    swap = pltpu.roll(jnp.where(low, b, a), HALF, 1)
    return [pltpu.bitcast(v, BF16).astype(F32) for v in (jnp.where(low, a, swap), jnp.where(low, swap, b))]


def _geglu(gate_up):
    g, u = gate_up[:HALF], gate_up[HALF:]
    return (g * u) * (1.0 + jnp.tanh(g * (GELU_LINEAR + g * g)))


class _Schedule:
    def __init__(self, table_ref, mark_ref):
        self.table_ref, self.mark_ref = table_ref, mark_ref
        self.steps, self.room, self.pending = [], [], {}
        self.slot = 0
        self.reset()

    def reset(self):
        self.token = self.last = self._never = self._zero = None

    def unpin(self):
        self.token = self.last = None

    @property
    def planned(self):
        return len(self.room)

    def add(self, room, fn, *args):
        self.room.extend(room)
        self.steps.append(functools.partial(fn, *args))

    def now(self, *pieces):
        self.steps.extend(pieces)

    def cut(self, *transfers):
        if transfers:
            self.now(self._block_end, *transfers)
        self.now(self._block_end)

    def _block_end(self):
        def tick(i, carry):
            self.mark_ref[0] = i
            return carry

        jax.lax.fori_loop(0, 2, tick, 0)
        self.reset()

    def spread(self, pieces, lo, hi):
        weight = np.cumsum(self.room[lo:hi])
        for n, piece in enumerate(pieces):
            at = int(np.searchsorted(weight, (n + 0.5) / len(pieces) * weight[-1]))
            self.pending.setdefault(lo + at, []).append(piece)

    def never(self):
        if self._never is None:
            self._never = self.table_ref[0:PACKED, :LANES].astype(F32)[:SUB] > 2.0
        return self._never

    def after(self, x):
        if self.token is None:
            return x
        token = self.token if self.token.dtype == x.dtype else pltpu.bitcast(self.token, x.dtype)
        if x.shape[0] == SUB:
            return jax.lax.select(self.never(), token, x)
        return jax.lax.select(self.never()[:1], token[:1], x)

    def zero(self):
        if self._zero is None:
            self._zero = jnp.where(self.never(), SUB, 0)[0, 0]
        return self._zero

    def dot(self, lhs, rhs):
        pieces = self.pending.pop(self.slot, ())
        for n, piece in enumerate(pieces):
            if self.last is not None:
                regs = self.last.shape[0] // SUB
                if regs <= PACKED:
                    row = (self.slot % 4 * len(pieces) + n) * regs // (4 * len(pieces)) * SUB
                else:
                    row = n * regs // len(pieces) * SUB
                self.token = self.last[row:row + SUB, :LANES]
            piece()
        self.slot += 1
        self.last = jnp.dot(lhs(), rhs(), preferred_element_type=F32)
        return self.last

    def run(self):
        for step in self.steps:
            step()
        assert not self.pending


def _kernel(q_hbm, k_hbm, v_hbm, taps_hbm, h_hbm, skip_hbm, wg_hbm, wu_hbm, wd_hbm,
            o_hbm,
            taps_v, skip_v, fwd_v, inv_v, q_v, k_v, v_v, h_v, wg_v, wu_v, wd_v, o_v,
            coef, spectra, h_prev, kv_s, y_freq, y_s, w_t, w_gu, wd_pair, wd_rest, x_s,
            h_ops, act_pair, act_rest, mark, sems):
    D = q_v.shape[0]
    DH, DQ = D // 2, D // 4
    taps = taps_v.shape[0]
    part = functools.partial
    plan = _Schedule(fwd_v, mark)
    dot, after = plan.dot, plan.after

    sem_ids, in_flight = {}, []

    def copies(name):
        kind, n = name[:2]
        every = slice(None)
        kv_pair = ((k_hbm, k_v), (v_hbm, v_v))
        if kind == "coefs":
            views = [(p, ...) for p in ((taps_hbm, taps_v), (skip_hbm, skip_v))]
        elif kind == "kv0":
            views = [(p, (slice(n * DQ, (n + 1) * DQ), slice(0, BLOCK))) for p in kv_pair]
        elif kind == "h0":
            views = [((h_hbm, h_v), (slice(n * DH, (n + 1) * DH), slice(0, BLOCK)))]
        elif kind == "kv":
            cols = slice(BLOCK, 2 * BLOCK) if n == 1 else slice(2 * BLOCK, None)
            views = [(p, (every, cols)) for p in kv_pair]
        elif kind == "h":
            views = [((h_hbm, h_v), (every, slice(n * BLOCK, (n + 1) * BLOCK)))]
        elif kind == "q":
            views = [((q_hbm, q_v), (every, slice(0, BLOCK) if n == 0 else slice(BLOCK, None)))]
        elif kind == "w":
            views = [(p, (every, slice(n * CHUNK, (n + 1) * CHUNK))) for p in ((wg_hbm, wg_v), (wu_hbm, wu_v))]
        elif kind == "wd":
            views = [((wd_hbm, wd_v), (every, every))]
        else:
            i, k = divmod(name[2], 2)
            col = n * BLOCK + k * CHUNK
            views = [((o_v, o_hbm), (slice(i * DH, (i + 1) * DH), slice(col, col + CHUNK)))]
        return [pltpu.make_async_copy(src.at[idx], dst.at[idx], sems.at[sem_ids.setdefault((name, i), len(sem_ids))])
                for i, ((src, dst), idx) in enumerate(views)]

    def start(*names):
        for name in names:
            in_flight.append(name)
            for copy in copies(name):
                copy.start()

    def wait(*names):
        for name in names:
            in_flight.remove(name)
            for copy in copies(name):
                copy.wait()

    def outputs(b):
        return [("out", b, m) for m in range(4)]

    def broadcast_coefs():
        rows = taps_v[...].astype(F32)
        for j in range(taps):
            coef[j] = jnp.broadcast_to(rows[j:j + 1], (LANES, D)).T
        coef[taps] = jnp.broadcast_to(skip_v[...].astype(F32).reshape(1, D), (LANES, D)).T

    def forward_table():
        n = jax.lax.broadcasted_iota(jnp.int32, (LANES, LANES), 0)
        k = jax.lax.broadcasted_iota(jnp.int32, (LANES, LANES), 1)
        angle = (((4 * k + 1) * n) & (4 * LANES - 1)).astype(F32) * (np.pi / (2 * LANES))
        fwd_v[:, :LANES] = jnp.cos(angle).astype(BF16)
        fwd_v[:, LANES:] = jnp.sin(angle).astype(BF16)

    def inverse_table():
        inv_v[...] = (fwd_v[...].astype(F32).T * (1.0 / LANES)).astype(BF16)

    def transpose_pieces(c, pin=False):
        def piece(m, i):
            w = (wg_v, wu_v)[m]
            groups = [w[u * HALF:(u + 1) * HALF, _tile(2 * c + i)] for pair in WEIGHT_TILES for u in pair]
            words = pltpu.bitcast(jnp.concatenate(groups, axis=0).T, U32)
            for j in range(len(WEIGHT_TILES)):
                w_t[c][m, i, j] = words[:, _tile(j)]
            if pin:
                plan.token = words[:SUB, :LANES]

        return [part(piece, m, i) for m in range(2) for i in range(2)]

    def gate_up_weight_pieces(c, pin=False):
        def piece(m, g, products):
            @functools.cache
            def raw(i, e, j):
                at = e * HALF // 2 + g * SUB
                if pin:
                    words = after(w_t[c][m, i, j, pl.ds(pl.multiple_of(at + plan.zero(), SUB), SUB)])
                else:
                    words = w_t[c][m, i, j, at:at + SUB]
                return pltpu.bitcast(words, BF16).astype(F32)

            for r in products:
                low = _low_lanes((PACKED, LANES))
                at = m * HALF // PACKED + g

                def padded(e, a, n):
                    j = 2 * (n % 2) + a
                    return jnp.where(low, raw(n // 2, e, j), 0.0) if j == 3 else raw(n // 2, e, j)

                if r in SHORT:
                    head = [_combine(LHS_TERMS[r], lambda n: raw(n // 2, e, (0, 2)[n % 2])) for e in range(2)]
                    tail = [_combine(LHS_TERMS[r], lambda n: raw(n // 2, e, (4, 3)[n % 2])) for e in range(2)]
                    tiles = [head[0] - jnp.where(low, 0.0, head[1]),
                             jnp.where(low, head[1], tail[1] - tail[0]),
                             jnp.where(low, tail[0], head[1])]
                else:
                    quads = [_combine(LHS_TERMS[r], part(padded, e, a)) for e in range(2) for a in range(2)]
                    tiles = [_combine(term, quads.__getitem__) for term in LHS_TERMS]
                w_gu[c][r][:, at:at + 1] = _fold_all(tiles)

        groups = range(HALF // PACKED)
        if pin:
            return [part(piece, m, g, rs) for m in range(2) for rs in ((2, 4), (1, 3), (0, 6), (5,)) for g in groups]
        return [part(piece, m, g, (r,)) for m in range(2) for g in groups for r in (0, 1, 3, 6, 5, 2, 4)]

    def down_weight_pieces(r):
        def rows(i, e, g):
            r0 = i * DH + e * DQ + PACKED * g
            return slice(r0, r0 + PACKED)

        def paired(j, g):
            scale = after(jnp.full((1, LANES), DOWN_SCALE, F32))

            def pick(e, n):
                i, f = divmod(n, 2)
                at = rows(i, e, g)
                return jnp.stack(_zip_halves(wd_v[at, _tile(4 * j + f)], wd_v[at, _tile(4 * j + 2 + f)]))

            left = [scale * _combine(LHS_TERMS[r], part(pick, e)) for e in range(2)]
            quads = [left[n // 2][n % 2] for n in range(4)]
            wd_pair[r][:, j, g:g + 1] = _fold_all([_combine(term, quads.__getitem__) for term in LHS_TERMS])

        def single(c, e):
            scale = after(jnp.full((1, LANES), DOWN_SCALE, F32))
            pick = lambda n: wd_v[pl.ds(n // 2 * DH + e * DQ, DQ), _tile(2 * c + n % 2)].astype(F32)
            wd_rest[r][c - 2 * PAIRS, e] = _fold(scale * _combine(LHS_TERMS[r], pick))

        return ([part(paired, j, g) for j in range(PAIRS) for g in range(DQ // PACKED)]
                + [part(single, c, e) for e in range(2) for c in range(2 * PAIRS, NUM_CHUNKS)])

    def kv_pieces(b, halves=(0, 1)):
        def piece(j, r0):
            rows = slice(r0, r0 + PACKED)
            lane = after(jax.lax.broadcasted_iota(jnp.int32, (SUB, LANES), 1))
            cur = pltpu.bitcast(k_v[rows, _tile(j)], U32)
            prev = pltpu.bitcast(k_v[rows, _tile(j - 1)], U32) if j else jnp.zeros_like(cur)
            shifted = pltpu.bitcast(cur, BF16).astype(F32) * coef[0, rows, :]
            for t in range(1, taps):
                moved = pltpu.roll(jnp.where(lane >= LANES - t, prev, cur), t, 1)
                shifted = shifted + pltpu.bitcast(moved, BF16).astype(F32) * coef[t, rows, :]
            kv_s[j, r0 // PACKED:r0 // PACKED + 1] = _fold(shifted * v_v[rows, _tile(j)].astype(F32))

        return [part(piece, 4 * b + n, i * DH + r0) for i in halves for n in range(4) for r0 in range(0, DH, PACKED)]

    def filter_spectra(b, i):
        rows = slice(i * DH, (i + 1) * DH)
        prev = (h_prev[b - 1, 0, rows, :], h_prev[b - 1, 1, rows, :]) if b else None
        for j in range(4 * b, 4 * b + 4):
            freq = dot(lambda: h_v[rows, _tile(j)], lambda: fwd_v[...])
            re, im = freq[:, :LANES], freq[:, LANES:]
            if j == 0:
                re = re + coef[taps, rows, :]
            c, d = (re + prev[1], im - prev[0]) if prev else (re, im)
            prev = (re, im)
            spectra[LAST - j, 0:3, rows, :] = jnp.stack([c, d - c, c + d])
        if b + 1 < NUM_BLOCKS:
            h_prev[b, 0, rows, :], h_prev[b, 1, rows, :] = prev

    def signal_spectra(b, i):
        rows = slice(i * DH, (i + 1) * DH)
        for j in range(4 * b, 4 * b + 4):
            freq = dot(lambda: _unfold(kv_s[j, i * DH // PACKED:(i + 1) * DH // PACKED]), lambda: fwd_v[...])
            re, im = freq[:, :LANES], freq[:, LANES:]
            spectra[j, 3, rows, :], spectra[j, 4, rows, :], spectra[j, 5, rows, :] = re + im, re, im

    def conv_pieces(b, halves=(0, 1)):
        state = {}

        def plane(hi, r0, p, js):
            rows = slice(r0, r0 + SUB)
            for n in (1, 0):
                out = hi - 1 + n
                j0, j1 = js[0], min(js[-1], out) + 1
                lags = spectra[LAST - out + j0:LAST - out + j1, p, rows, :]
                total = jnp.sum(lags * spectra[j0:j1, 3 + p, rows, :], axis=0)
                if j0 or p:
                    base = after(state[n] if j0 else state["shared", n])
                    state[n] = base - total if p == 2 else base + total
                else:
                    state[n] = after(total)
                if js[-1] == hi and p:
                    y_freq[out, rows, _tile(2 - p)] = state[n].astype(BF16)
                elif js[-1] == hi:
                    state["shared", n] = state[n]

        runs = lambda hi: [range(hi + 1)] if hi < 8 else [range((hi + 1) // 2), range((hi + 1) // 2, hi + 1)]
        return [part(plane, hi, r0, p, js) for i in halves for hi in (4 * b + 1, 4 * b + 3)
                for r0 in range(i * DH, (i + 1) * DH, SUB) for p in range(3) for js in runs(hi)]

    def inverse(b, i):
        rows = slice(i * DH, (i + 1) * DH)
        for j in range(4 * b, 4 * b + 4):
            y_s[b][j % 4, rows, :] = dot(lambda: y_freq[j, rows, :], lambda: inv_v[...])

    def norm_pieces(b, layer):
        state = {}

        def fetch(stage, t, r0, size):
            if layer == 0 and stage < 3:
                return q_v[r0:r0 + size, _tile(4 * b + t)].astype(F32)
            if (b, layer) == (0, 0):
                return x_s[b][r0:r0 + size, _tile(t)]
            return x_s[b][pl.ds(pl.multiple_of(r0 + stage * plan.zero(), SUB), size), _tile(t)]

        def average(t, r0, val):
            val = jnp.concatenate([state["sum", t], val], axis=0) if r0 else val
            state["sum", t] = jnp.sum(val.reshape(-1, SUB, LANES), axis=0)
            return jnp.sum(state["sum", t], axis=0, keepdims=True) * (1.0 / D) if r0 + HALF == D else None

        def center(t, r0):
            x = fetch(0, t, r0, HALF)
            state["mean", t] = average(t, r0, jnp.concatenate([after(x[:SUB]), x[SUB:]], axis=0))

        def deviation(stage, t, r0):
            centered = fetch(stage, t, r0, HALF) - after(state["mean", t])
            var = average(t, r0, centered * centered)
            if var is not None:
                state["scale", t] = jax.lax.rsqrt(var + EPS) * (GELU_SCALE if stage == 3 else 1.0)

        def gate(t, r0):
            rows = slice(r0, r0 + HALF)
            x = fetch(2, t, r0, HALF)
            x = x + (x - after(state["mean", t])) * state["scale", t] * y_s[b][t, rows, :]
            x_s[b][rows, _tile(t)] = x
            mean = average(t, r0, x)
            if mean is not None:
                state["mean", t] = mean

        def operands(u, r0, products):
            mean = functools.cache(lambda t: after(state["mean", t]))
            at = (u * HALF + r0) // PACKED

            @functools.cache
            def normed(j, a, t):
                row = (4 * j + 2 * a + u) * HALF + r0
                return (fetch(4 + products[0], t, row, PACKED) - mean(t)) * state["scale", t] if row < D else None

            for r in products:
                right = lambda a, t: _combine(RHS_TERMS[r], lambda n: normed(n // 2, a, 2 * (n % 2) + t))
                if r in SHORT:
                    for t in range(2):
                        for a in range(2 - u):
                            h_ops[RHS_START[r] + 2 * t + a, at:at + 1] = _fold(right(a, t))
                else:
                    quads = [right(a, t) for a in range(2) for t in range(2)]
                    h_ops[RHS_START[r]:RHS_START[r] + 7, at:at + 1] = _fold_all(
                        [_combine(term, quads.__getitem__) for term in RHS_TERMS])

        stages = (center, part(deviation, 1), gate, part(deviation, 3))
        return ([part(stage, t, r0) for stage in stages for t in range(4) for r0 in range(0, D, HALF)],
                [part(operands, u, r0, rs) for rs in ((0,), (1, 3), (5,), (2,), (4, 6))
                 for u in range(2) for r0 in range(0, HALF, PACKED)])

    def gate_up(c, defer):
        def product(r):
            lhs = _load_tiles(w_gu[c][r], ...)
            at = RHS_START[r]
            if r not in SHORT:
                rhs = _load_tiles(h_ops, slice(at, at + 7))
                return _inner_sum(lambda s: dot(part(lhs, s), part(rhs, s)))
            out = [None] * 4
            for t in range(2):
                first, second = at + 2 * t, at + 2 * t + 1
                join = lambda a, b: _unfold(jnp.concatenate([a, b], axis=0))
                shared = dot(part(lhs, 2), lambda: join(h_ops[second, 0:4], h_ops[first, 4:8]))
                out[t] = dot(part(lhs, 0), lambda: _unfold(h_ops[first])) + shared
                out[2 + t] = dot(part(lhs, 1), lambda: join(h_ops[first, 0:4], h_ops[second, 0:4])) + shared
            return out

        acts = {}
        _outer_sum(product, GATE_UP_ORDER, lambda m, blocks: acts.update({m: [_geglu(v) for v in blocks]}))

        def operands(r, g0, g1, late):
            def quadrant(n, m):
                x = acts[m ^ 1][n][PACKED * g0:PACKED * g1]
                if late and m == RHS_TERMS[r][0]:
                    x = jnp.concatenate([after(x[i:i + SUB]) for i in range(0, x.shape[0], SUB)], axis=0)
                return x

            right = [_combine(RHS_TERMS[r], part(quadrant, n)) for n in range(4)]
            if c < 2 * PAIRS:
                at = 4 * (c % 2)
                act_pair[c // 2][r, :, at + g0:at + g1] = _fold_all(
                    [_combine(term, right.__getitem__) for term in RHS_TERMS])
            else:
                for n in range(4):
                    at = 4 * (n // 2)
                    act_rest[c - 2 * PAIRS][r, n % 2, at + g0:at + g1] = _fold(right[n])

        for r in range(7):
            if r not in defer:
                operands(r, 0, 4, False)
        if defer:
            plan.spread([part(operands, r, g, g + 1, True) for r in defer for g in range(4)],
                        plan.slot + 2, plan.slot + 9)

    def down(b, layer):
        def product(r):
            lhs = [_load_tiles(wd_pair[r], (slice(None), j)) for j in range(PAIRS)]
            rhs = [_load_tiles(act_pair[j], r) for j in range(PAIRS)]
            one = lambda s, j: dot(part(lhs[j], s), part(rhs[j], s))
            out = _inner_sum(lambda s: functools.reduce(jnp.add, [one(s, j) for j in range(PAIRS)]))
            lhs_rest = [_load_tiles(wd_rest[r], c) for c in range(len(act_rest))]
            rhs_rest = [_load_tiles(ref, r) for ref in act_rest]
            rest = lambda n, c: dot(part(lhs_rest[c], n // 2), part(rhs_rest[c], n % 2))
            return [functools.reduce(jnp.add, [out[n]] + [rest(n, c) for c in range(len(act_rest))]) for n in range(4)]

        end = plan.slot + 7 * DOWN_PASSES

        def emit(m, blocks):
            for n, val in enumerate(blocks):
                r0 = (m // 2) * DH + (n // 2) * DQ
                rows, t = slice(r0, r0 + DQ), 2 * (1 - m % 2) + n % 2
                val = x_s[b][rows, _tile(t)] + val
                if layer == 0:
                    x_s[b][rows, _tile(t)] = val
                else:
                    o_v[rows, _tile(4 * b + t)] = val.astype(BF16)
            if layer == 1 and b == NUM_BLOCKS - 1:
                if plan.slot < end:
                    plan.pending.setdefault(plan.slot + 8, []).append(part(start, ("out", b, m ^ 1)))
                else:
                    start(("out", b, m ^ 1))

        _outer_sum(product, DOWN_ORDER, emit)

    def add_gate_up(chunks=range(NUM_CHUNKS), busy=0.1):
        lo = plan.planned
        room = [busy if 9 <= i < 15 or 22 <= i < 28 or i >= 35 else 1.0 for i in range(GATE_UP_PASSES)]
        for c in chunks:
            plan.add(room, gate_up, c, () if c + 1 == NUM_CHUNKS else (3, 6))
        return lo, plan.planned

    def add_down(b, layer):
        lo = plan.planned
        plan.add([1.0] * (7 * DOWN_PASSES), down, b, layer)
        return lo, plan.planned

    def add_transform(fn, b, halves=(0, 1)):
        lo = plan.planned
        for i in halves:
            plan.add([4.0] * 4, fn, b, i)
        return lo, plan.planned

    def spread_norm(b, layer, lo, hi):
        stats, ops = norm_pieces(b, layer)
        mid = lo + int((hi - lo) * 0.62)
        plan.spread(stats, lo, mid)
        plan.spread(ops, mid, hi)

    def send(b, job):
        plan.spread([part(start, *outputs(b))], job[0] + 8, job[0] + 9)

    plan.now(part(start, ("coefs", 0), ("h0", 0), ("kv0", 0), ("kv0", 1), ("h0", 1), ("kv0", 2),
                  ("kv0", 3), ("q", 0), ("h", 1), *[("w", c) for c in range(NUM_CHUNKS)], ("wd", 0), ("kv", 1),
                  ("h", 2), ("h", 3), ("kv", 2), ("q", 1)),
             forward_table, part(wait, ("coefs", 0)), broadcast_coefs, inverse_table)
    plan.cut(part(wait, ("h0", 0)))
    add_transform(filter_spectra, 0, [0])
    plan.now(part(wait, ("kv0", 0), ("kv0", 1)), *kv_pieces(0, [0]))
    add_transform(signal_spectra, 0, [0])
    plan.cut(part(wait, ("h0", 1)))
    plan.spread(conv_pieces(0, [0]), *add_transform(filter_spectra, 0, [1]))
    plan.now(part(wait, ("kv0", 2), ("kv0", 3)), *kv_pieces(0, [1]))
    add_transform(signal_spectra, 0, [1])
    plan.cut()
    plan.spread(conv_pieces(0, [1]), *add_transform(inverse, 0, [0]))
    plan.now(part(wait, ("q", 0)))
    stats, ops = norm_pieces(0, 0)
    plan.spread(stats[:56], *add_transform(inverse, 0, [1]))
    plan.now(plan.unpin, *stats[56:77])
    plan.cut(part(wait, ("h", 1)))
    plan.spread(stats[77:] + ops[:8], *add_transform(filter_spectra, 1))
    plan.now(part(wait, ("w", 0)), plan.unpin, *ops[8:16])
    for n, piece in enumerate(transpose_pieces(0, pin=True)):
        plan.now(piece, *ops[16 + 6 * n:22 + 6 * n])
    plan.now(plan.unpin, *gate_up_weight_pieces(0))

    for chunks, arrivals, prepare in (((0,), (1,), (1,)), ((1,), (2, 3), (2,)), ((2,), (4, 5), (3, 4)),
                                      ((3, 4), (6,), (5, 6))):
        plan.cut(part(wait, *[("w", n) for n in arrivals]))
        lo, hi = add_gate_up(chunks, busy=0.4)
        if prepare[0] in arrivals:
            plan.spread(transpose_pieces(prepare[0]), lo, lo + 2)
            lo += 5
        plan.spread([piece for n in prepare for piece in gate_up_weight_pieces(n, pin=n in arrivals)], lo, hi - 1)
        plan.spread([piece for n in arrivals if n > prepare[0] for piece in transpose_pieces(n)], lo,
                    lo + 20 if len(prepare) > 1 else hi - 2)
    plan.cut(part(wait, ("wd", 0)))
    lo, hi = add_gate_up((5, 6))
    plan.spread([piece for r in DOWN_ORDER[:4] for piece in down_weight_pieces(r)], lo, hi - 1)
    plan.cut(part(wait, ("kv", 1), ("h", 2), ("h", 3)))
    lo, hi = add_down(0, 0)
    for n, r in enumerate(DOWN_ORDER[4:]):
        plan.spread(down_weight_pieces(r), lo + n * DOWN_PASSES, lo + (n + 1) * DOWN_PASSES)
    plan.spread(kv_pieces(1), lo + DOWN_PASSES, lo + 5 * DOWN_PASSES + 10)
    add_transform(filter_spectra, 2)
    add_transform(filter_spectra, 3)
    add_transform(signal_spectra, 1)
    stats, ops = norm_pieces(0, 1)
    plan.spread([piece for piece in stats if piece.args[-2] < 2], lo + 5 * DOWN_PASSES + 5, hi + 3)
    plan.spread([piece for piece in stats if piece.args[-2] >= 2], hi + 1, hi + 15)
    plan.spread(ops, hi + 15, plan.planned - 1)

    plan.cut(part(wait, ("kv", 2), ("q", 1)))
    lo, _ = add_gate_up()
    add_transform(signal_spectra, 2)
    plan.spread(kv_pieces(2), lo, lo + 2 * GATE_UP_PASSES)
    plan.spread(conv_pieces(1), lo + 2 * GATE_UP_PASSES, plan.planned)
    plan.cut()
    inv = add_transform(inverse, 1)
    _, hi = add_down(0, 1)
    spread_norm(1, 0, inv[1], hi - 12)
    conv = conv_pieces(2)
    split = len(conv) // 5 // 6 * 6
    plan.spread(conv[:split], inv[0], hi)

    plan.cut()
    job = add_gate_up()
    plan.spread(conv[split:], *job)
    send(0, job)
    inv = add_transform(inverse, 2)
    lo, hi = add_down(1, 0)
    add_transform(signal_spectra, 3)
    spread_norm(2, 0, inv[1], hi + 8)
    plan.spread(kv_pieces(3, [0]), inv[0], lo + 30)
    plan.spread(kv_pieces(3, [1]), lo + 30, hi)

    plan.cut()
    conv = conv_pieces(3)
    split = 2 * len(conv) // 5 // 6 * 6
    plan.spread(conv[:split], *add_gate_up())
    lo, hi = add_down(2, 0)
    spread_norm(1, 1, lo, hi - 12)
    plan.spread(conv[split:-split], lo, hi)
    plan.spread(conv[-split:], *add_gate_up())
    inv = add_transform(inverse, 3)
    _, hi = add_down(1, 1)
    spread_norm(3, 0, inv[1], hi - 12)

    plan.cut()
    send(1, add_gate_up())
    lo, hi = add_down(3, 0)
    spread_norm(2, 1, lo, hi - 12)
    add_gate_up()
    lo, hi = add_down(2, 1)
    spread_norm(3, 1, lo, hi - 12)
    send(2, add_gate_up())
    add_down(3, 1)
    plan.now(part(wait, *[name for b in range(NUM_BLOCKS) for name in outputs(b)]))

    plan.run()
    assert not in_flight


def _run(A_q, A_k, A_v, A_shift_k, A_ssm_k, A_ssm_D, B_x, B_w_gate, B_w_up, B_w_down):
    del B_x
    batch, S, D = A_q.shape
    F = B_w_gate.shape[1]
    taps = A_shift_k.shape[1]
    assert (batch, S, D, F) == (1, NUM_BLOCKS * BLOCK, 7 * HALF, NUM_CHUNKS * CHUNK)
    tiles, rest = S // LANES, NUM_CHUNKS - 2 * PAIRS
    hbm = pl.BlockSpec(memory_space=pltpu.HBM)
    folded = lambda *lead: pltpu.VMEM(lead + (SUB, 2 * LANES), BF16)
    out = pl.pallas_call(
        _kernel,
        out_shape=jax.ShapeDtypeStruct((D, S), BF16),
        in_specs=[hbm] * 9,
        out_specs=hbm,
        scratch_shapes=[
            *[pltpu.VMEM(shape, BF16) for shape in ((taps, D), (D,), (LANES, 2 * LANES), (2 * LANES, LANES))],
            *[pltpu.VMEM((D, S), BF16)] * 4,
            *[pltpu.VMEM((D, F), BF16)] * 3,
            pltpu.VMEM((D, S), BF16),
            pltpu.VMEM((taps + 1, D, LANES), F32),
            pltpu.VMEM((tiles, 6, D, LANES), F32),
            pltpu.VMEM((NUM_BLOCKS - 1, 2, D, LANES), F32),
            folded(tiles, D // PACKED),
            pltpu.VMEM((tiles, D, 2 * LANES), BF16),
            [pltpu.VMEM((4, D, LANES), F32)] * NUM_BLOCKS,
            [pltpu.VMEM((2, 2, len(WEIGHT_TILES), HALF, LANES), U32)] * NUM_CHUNKS,
            [[folded(3 if r in SHORT else 7, SUB) for r in range(7)]] * NUM_CHUNKS,
            [folded(7, PAIRS + 1, D // 4 // PACKED)] * 7,
            [folded(rest, 2, D // 4 // PACKED)] * 7,
            [pltpu.VMEM((D, BLOCK), F32)] * NUM_BLOCKS,
            folded(RHS_START[7], SUB),
            [folded(7, 7, SUB)] * PAIRS,
            [folded(7, 2, SUB)] * rest,
            pltpu.SMEM((1,), jnp.int32),
            pltpu.SemaphoreType.DMA((56,)),
        ],
        compiler_params=pltpu.CompilerParams(
            vmem_limit_bytes=120 * 2**20, disable_bounds_checks=True, disable_semaphore_checks=True),
    )(A_q[0].T, A_k[0].T, A_v[0].T, A_shift_k.T, A_ssm_k, A_ssm_D, B_w_gate, B_w_up, B_w_down.T)
    return out.T[None]


@jax.jit
def pallas_interleave_layers__ssm_conv_h3__geglu_ffn__prompt_kernel(
    A_q: jax.Array,
    A_k: jax.Array,
    A_v: jax.Array,
    A_shift_k: jax.Array,
    A_ssm_k: jax.Array,
    A_ssm_D: jax.Array,
    B_x: jax.Array,
    B_w_gate: jax.Array,
    B_w_up: jax.Array,
    B_w_down: jax.Array,
):
    return _run(A_q, A_k, A_v, A_shift_k, A_ssm_k, A_ssm_D, B_x, B_w_gate, B_w_up, B_w_down)
```
